```python
import jax
import jax.numpy as jnp

def _softmax(x, axis=-1):
    return jax.nn.softmax(x, axis=axis)
def _gelu(x):
    return jax.nn.gelu(x, approximate=True)
def _silu(x):
    return jax.nn.silu(x)
def _sigmoid(x):
    return jax.nn.sigmoid(x)
def _layernorm(x, axis=-1, eps=1e-5):
    m = jnp.mean(x, axis=axis, keepdims=True)
    v = jnp.var(x, axis=axis, keepdims=True)
    return (x - m) / jnp.sqrt(v + eps)
def _scatter_add(tgt, idx, src, axis=0):
    return tgt.at[idx].add(src)
def _segment_sum(src, seg, n):
    return jax.ops.segment_sum(src, seg, n)
class _Rng:
    def __init__(self, key):
        self._k = key
    def _next(self):
        self._k, sub = jax.random.split(self._k)
        return sub
    def normal(self, shape):
        return jax.random.normal(self._next(), shape, dtype=jnp.bfloat16)
    def randint(self, lo, hi, shape):
        return jax.random.randint(self._next(), shape, lo, hi, dtype=jnp.int32)
    def uniform(self, shape, lo=0.0, hi=1.0):
        return jax.random.uniform(self._next(), shape, jnp.bfloat16, lo, hi)
    def permutation(self, n):
        return jax.random.permutation(self._next(), n)


kernel_name = 'standalone__self_sup_conv_stem_wavlm__speech'

def setup_inputs():
    _rng = _Rng(jax.random.key(int.from_bytes(__import__("os").urandom(4), "little")))
    _w = (lambda a: (lambda t: t.astype(jnp.bfloat16) if jnp.issubdtype(t.dtype, jnp.floating) else t)(jnp.asarray(a)))
    B, T, D, K = 2, 16000, 512, 31
    scale = (K * D) ** -0.5
    return {
        "x": _w((lambda *s: _rng.normal(s) * 0.05)(B, T, D)),
        "w": _w((lambda *s: _rng.normal(s) * 0.05)(K, D, D) * scale),
        "gn_gamma": _w((lambda *s: _rng.normal(s) * 0.05)(D) * 0.1 + 1.0),
        "gn_beta": _w((lambda *s: _rng.normal(s) * 0.05)(D) * 0.1),
    }

def reference(x, w, gn_gamma, gn_beta):
    B, T, D = x.shape
    K = w.shape[0]
    s = 2
    L = (T - K) // s + 1
    h = jnp.einsum('blc,cd->bld', x[:, 0:s * L:s, :], w[0])
    for i in range(1, K):
        h = h + jnp.einsum('blc,cd->bld', x[:, i:i + s * L:s, :], w[i])
    mu = jnp.einsum('bld->bd', h)[:, None, :] / L
    var = jnp.einsum('bld->bd', (h - mu) ** 2)[:, None, :] / L
    h = (h - mu) / jnp.sqrt(var + 1e-5)
    h = h * gn_gamma[None, None, :] + gn_beta[None, None, :]
    return _gelu(h)
```

```python
import math
import functools
import jax
import jax.numpy as jnp
from jax import lax
from jax.experimental import pallas as pl
from jax.experimental.pallas import tpu as pltpu

class _Node:
    __slots__ = ("op", "args", "c", "idx")

class _Prog:
    def __init__(self):
        self.nodes = []
        self.cse = {}

    def _mk(self, op, args=(), c=None):
        key = (op, tuple(a.idx for a in args), c)
        n = self.cse.get(key)
        if n is None:
            n = _Node()
            n.op, n.args, n.c, n.idx = op, args, c, len(self.nodes)
            self.nodes.append(n)
            self.cse[key] = n
        return n

    def inp(self, i):
        return (1, self._mk("in", (), i))

    def neg(self, a):
        return None if a is None else (-a[0], a[1])

    def add(self, a, b):
        if a is None:
            return b
        if b is None:
            return a
        (sa, na), (sb, nb) = a, b
        if sa == sb:
            if na is nb:
                return (sa, self._mk("mul", (na,), 2.0))
            x, y = sorted((na, nb), key=lambda n: n.idx)
            return (sa, self._mk("add", (x, y)))
        if na is nb:
            return None
        if sa > 0:
            return (1, self._mk("sub", (na, nb)))
        return (1, self._mk("sub", (nb, na)))

    def sub(self, a, b):
        return self.add(a, self.neg(b))

    def mul(self, a, c):
        if a is None or abs(c) < 1e-12:
            return None
        if abs(c - 1) < 1e-12:
            return a
        if abs(c + 1) < 1e-12:
            return self.neg(a)
        return (a[0] * (1 if c > 0 else -1), self._mk("mul", (a[1],), abs(float(c))))


def _cadd(B, a, b): return (B.add(a[0], b[0]), B.add(a[1], b[1]))
def _csub(B, a, b): return (B.sub(a[0], b[0]), B.sub(a[1], b[1]))
def _cconj(B, a): return (a[0], B.neg(a[1]))
def _cmuli(B, a): return (B.neg(a[1]), a[0])
def _cmulni(B, a): return (a[1], B.neg(a[0]))


def _ctw(B, a, k, n):
    k %= n
    if k == 0:
        return a
    if 2 * k == n:
        return (B.neg(a[0]), B.neg(a[1]))
    if 4 * k == n:
        return _cmulni(B, a)
    if 4 * k == 3 * n:
        return _cmuli(B, a)
    th = -2 * math.pi * k / n
    c, s = math.cos(th), math.sin(th)
    if (8 * k) % n == 0:
        m = abs(c)
        f = lambda v, sg: v if sg > 0 else B.neg(v)
        re = B.sub(f(a[0], c), f(a[1], s))
        im = B.add(f(a[1], c), f(a[0], s))
        return (B.mul(re, m), B.mul(im, m))
    return (B.sub(B.mul(a[0], c), B.mul(a[1], s)), B.add(B.mul(a[1], c), B.mul(a[0], s)))


def _rdft(B, x):
    n = len(x)
    if n == 1:
        return [(x[0], None)]
    if n == 2:
        return [(B.add(x[0], x[1]), None), (B.sub(x[0], x[1]), None)]
    E = _rdft(B, x[0::2]); O1 = _rdft(B, x[1::4]); O3 = _rdft(B, x[3::4])
    X = [None] * n
    q = n // 4
    for k in range(0, q // 2 + 1):
        if k >= q:
            break
        a = _ctw(B, O1[k], k, n); b = _ctw(B, O3[k], 3 * k, n)
        s = _cadd(B, a, b); d = _cmuli(B, _csub(B, a, b))
        X[k] = _cadd(B, E[k], s)
        X[k + 2 * q] = _csub(B, E[k], s)
        X[k + q] = _csub(B, E[k + q], d)
        X[k + 3 * q] = _cadd(B, E[k + q], d)
    for k in range(n):
        if X[k] is None:
            X[k] = _cconj(B, X[n - k])
    return X


NF = 32


def _spectrum(B, x):
    X = _rdft(B, x)
    o = []
    for k in range(1, NF // 2):
        o += [X[k][0], X[k][1]]
    return o + [X[0][0], X[NF // 2][0]]


def data_program():
    B = _Prog()
    o = _spectrum(B, [B.inp(i) for i in range(NF)])
    outs = []
    for f in range(15):
        outs += [B.add(o[2 * f], o[2 * f + 1]), o[2 * f], o[2 * f + 1]]
    outs += [None, o[30], o[31]]
    return B, outs


def weight_program(ntaps):
    B = _Prog()
    o = _spectrum(B, [B.inp(i) if i < ntaps else None for i in range(NF)])
    outs = []
    for f in range(15):
        vr, vi = o[2 * f], B.neg(o[2 * f + 1])
        outs += [vr, B.sub(vi, vr), B.add(vr, vi)]
    outs += [None, B.mul(o[30], 0.5), B.mul(o[31], -0.5)]
    return B, outs


def output_program(nout):
    F = _Prog()
    o = _spectrum(F, [F.inp(i) if i < nout else None for i in range(NF)])
    B = _Prog()
    order = list(range(30)) + [31, 30]
    adj = {}
    def push(term, val):
        if term is None or val is None:
            return
        adj.setdefault(term[1].idx, []).append(val if term[0] > 0 else B.neg(val))
    for slot, k in enumerate(order):
        push(o[k], B.inp(slot))
    res = [None] * nout
    for n in reversed(F.nodes):
        terms = adj.get(n.idx)
        if not terms:
            continue
        a = terms[0]
        for t in terms[1:]:
            a = B.add(a, t)
        if n.op == "in":
            res[n.c] = a
        elif n.op == "add":
            push((1, n.args[0]), a); push((1, n.args[1]), a)
        elif n.op == "sub":
            push((1, n.args[0]), a); push((-1, n.args[1]), a)
        else:
            push((1, n.args[0]), B.mul(a, n.c))
    return B, res


def run_program(prog, inputs):
    B, outs = prog
    memo = {}
    get = inputs if callable(inputs) else inputs.__getitem__
    def ev(n):
        v = memo.get(n.idx)
        if v is None:
            if n.op == "in":
                v = get(n.c)
            elif n.op == "add":
                v = ev(n.args[0]) + ev(n.args[1])
            elif n.op == "sub":
                v = ev(n.args[0]) - ev(n.args[1])
            else:
                v = ev(n.args[0]) * n.c
            memo[n.idx] = v
        return v
    res = []
    for o in outs:
        if o is None:
            res.append(None)
        else:
            res.append((o[0], ev(o[1])))
    return res


def count_ops(prog):
    B, outs = prog
    seen = set(); st = [o[1] for o in outs if o is not None]; c = 0
    while st:
        n = st.pop()
        if n.idx in seen:
            continue
        seen.add(n.idx)
        c += n.op != "in"
        st.extend(n.args)
    return c


_DATA = data_program()
_WPROG = (weight_program(16), weight_program(15))
_S = 17
_OUT = output_program(_S)

_M = 96
_NC = 5
_CR = _M * _S
_HR = _NC * _CR
_XW = 1648
_NI = 8
_NP = 48


def _signed(t):
    return None if t is None else (t[1] if t[0] > 0 else -t[1])


def _kernel(x_hbm, w_hbm, g_ref, be_ref, o_ref,
            xs, wst, wc, dc, oc, h, st, ab, xsem, wsem, *, B, T, L):
    t = pl.program_id(0)
    NQ = B * _NC
    xw = xs.bitcast(jnp.uint32)

    def x_copy(q, lt, rows):
        slot = q % 2
        b = q // _NC
        c = q % _NC
        r0 = pl.multiple_of(c * (2 * _CR), 16)
        return pltpu.make_async_copy(
            x_hbm.at[b, pl.ds(r0, rows), pl.ds(lt * 128, 128)],
            xs.at[slot, lt, pl.ds(0, rows)], xsem.at[slot])

    last_rows = T - (_NC - 1) * 2 * _CR

    def x_start(q):
        is_last = (q % _NC) == _NC - 1
        @pl.when(is_last)
        def _():
            for lt in range(4):
                x_copy(q, lt, last_rows).start()
            z = jnp.zeros((2 * _XW - last_rows, 128), jnp.bfloat16)
            for lt in range(4):
                xs[q % 2, lt, pl.ds(last_rows, 2 * _XW - last_rows), :] = z
        @pl.when(jnp.logical_not(is_last))
        def _():
            for lt in range(4):
                x_copy(q, lt, 2 * _XW).start()

    def x_wait(q):
        is_last = (q % _NC) == _NC - 1
        @pl.when(is_last)
        def _():
            for lt in range(4):
                x_copy(q, lt, last_rows).wait()
            lw = last_rows // 2
            for lt in range(4):
                v = xw[q % 2, lt, pl.ds(lw - 8, 8), :]
                row = lax.broadcasted_iota(jnp.int32, (8, 128), 0)
                xw[q % 2, lt, pl.ds(lw - 8, 8), :] = jnp.where(row == 7, v & jnp.uint32(0xFFFF), v)
        @pl.when(jnp.logical_not(is_last))
        def _():
            for lt in range(4):
                x_copy(q, lt, 2 * _XW).wait()

    def w_copy(s, lt):
        return pltpu.make_async_copy(
            w_hbm.at[:, pl.ds(s * 32, 32), pl.ds(lt * 128, 128)],
            wst.at[s % 2, lt], wsem.at[s % 2])

    def w_unit(s, rg, lt):
        for ph in range(2):
            prog = _WPROG[ph]
            ld = lambda j: wst[s % 2, lt, 2 * j + ph, pl.ds(pl.multiple_of(rg * 16, 16), 16), :].astype(jnp.float32)
            res = run_program(prog, ld)
            r0 = pl.multiple_of(ph * 512 + s * 32 + rg * 16, 16)
            for p, (rv, dv) in enumerate(zip(res, _DATA[1])):
                if rv is None:
                    continue
                v = rv[1] if rv[0] * dv[0] > 0 else -rv[1]
                wc[p, lt, pl.ds(r0, 16), :] = v.astype(jnp.bfloat16)

    def d_unit(slot, g, lt, ph):
        sub = xw.at[slot, lt, pl.ds(pl.multiple_of(g * (16 * _S), 16), 288)]
        def ld(j):
            w = jnp.concatenate([sub[pl.ds(j, 8, stride=2 * _S), :],
                                 sub[pl.ds(_S + j, 8, stride=2 * _S), :]], axis=0)
            w = (w << 16) if ph == 0 else (w & jnp.uint32(0xFFFF0000))
            return pltpu.bitcast(w, jnp.float32)
        res = run_program(_DATA, ld)
        for p, rv in enumerate(res):
            if rv is not None:
                dc[slot, p, ph * 4 + lt, pl.ds(pl.multiple_of(g * 16, 16), 16), :] = rv[1].astype(jnp.bfloat16)

    def m_bin(slot, f):
        for lt in range(4):
            k = []
            for c in range(3):
                p = 3 * f + c
                lhs = jnp.concatenate([dc[slot, p, kt] for kt in range(8)], axis=1)
                k.append(jnp.dot(lhs, wc[p, lt], preferred_element_type=jnp.float32))
            oc[slot, 2 * f, lt] = k[0] - k[2]
            oc[slot, 2 * f + 1, lt] = k[0] + k[1]

    def o_unit(slot, q, g8, lt):
        b = q // _NC
        c = q % _NC
        ld = lambda k: oc[slot, k, lt, pl.ds(pl.multiple_of(g8 * 8, 8), 8), :]
        res = run_program(_OUT, ld)
        blk0 = c * _M + (g8 // 2) * 16
        odd = g8 % 2
        base = pl.multiple_of(blk0 * _S, 8)
        sub = h.at[b, lt, pl.ds(base, 16 * _S)]
        blk = blk0 + odd + 2 * lax.broadcasted_iota(jnp.int32, (8, 128), 0)
        nfull = L // _S
        jr = L - nfull * _S
        m_lo = jnp.where(blk <= nfull, 1.0, 0.0).astype(jnp.float32)
        m_hi = jnp.where(blk < nfull, 1.0, 0.0).astype(jnp.float32)
        s = None; sq = None
        ys = []
        for j, rv in enumerate(res):
            y = _signed(rv)
            ys.append(y)
            ym = y * (m_lo if j < jr else m_hi)
            s = ym if s is None else s + ym
            sq = ym * ym if sq is None else sq + ym * ym
        st[b, 0, lt] += s
        st[b, 1, lt] += sq
        return sub, odd, ys

    def o_store(sub, odd_static, ys):
        for j, y in enumerate(ys):
            sub[pl.ds(odd_static * _S + j, 8, stride=2 * _S), :] = y

    def stats(b):
        for lt in range(4):
            s = jnp.sum(st[b, 0, lt], axis=0, keepdims=True) * (1.0 / L)
            q = jnp.sum(st[b, 1, lt], axis=0, keepdims=True) * (1.0 / L)
            var = jnp.maximum(q - s * s, 0.0) * (1.0 / 256.0)
            a = lax.rsqrt(var + 1e-5) * (1.0 / 16.0) * g_ref[:, lt * 128:(lt + 1) * 128].astype(jnp.float32)
            bb = be_ref[:, lt * 128:(lt + 1) * 128].astype(jnp.float32) - s * a
            ab[0, lt] = jnp.broadcast_to(a, (8, 128))
            ab[1, lt] = jnp.broadcast_to(bb, (8, 128))

    ou = o_ref.bitcast(jnp.uint32)

    def gelu_norm(b, lt, rows):
        z = h[b, lt, rows, :] * ab[0, lt] + ab[1, lt]
        u = z * (0.7978845608028654 + 0.035677408136300125 * (z * z))
        return (0.5 * z) * (1.0 + jnp.tanh(u))

    def e_part(final, c, i):
        if not final:
            lt = i % 4
            for r in range(102):
                rows = pl.ds(pl.multiple_of(c * _CR + ((i // 4) * 102 + r) * 8, 8), 8)
                h[0, lt, rows, :] = gelu_norm(0, lt, rows)
            return
        g0 = jnp.minimum(26 * i, _CR // 8 - 26)
        for r in range(26):
            rl = pl.multiple_of((g0 + r) * 8, 8)
            rows = pl.ds(pl.multiple_of(c * _CR + rl, 8), 8)
            if True:
                wv = [pltpu.pack_elementwise([h[0, lt, rows, :], gelu_norm(1, lt, rows)],
                                             packed_dtype=jnp.bfloat16) for lt in range(4)]
                ou[pl.ds(rl, 8), 0, :] = jnp.concatenate(wv, axis=1)

    def step(D, Mm, O, E):
        def body(i, carry):
            lt = i % 4
            hi = i // 4
            if D:
                for k in range(3):
                    for ph in range(2):
                        d_unit(t % 2, hi * 3 + k, lt, ph)
            if Mm:
                for k in range(2):
                    m_bin((t + 1) % 2, 2 * i + k)
            if O:
                for k in range(6):
                    g8 = hi * 6 + k
                    sub, odd, ys = o_unit(t % 2, t - 2, g8, lt)
                    o_store(sub, k % 2, ys)
            if E:
                e_part(not (D or Mm or O), ec, i)
            return carry
        lax.fori_loop(0, _NI, body, 0)

    ec = jnp.where(t < 2 * _NC + 2, t - (_NC + 2), t - (2 * _NC + 2))

    @pl.when(t == 0)
    def _():
        x_start(0)
        for lt in range(4):
            w_copy(0, lt).start()
        st[...] = jnp.zeros(st.shape, jnp.float32)
        zc = jnp.zeros((1024, 128), jnp.bfloat16)
        for lt in range(4):
            wc[45, lt] = zc
        for s in range(16):
            if s + 1 < 16:
                for lt in range(4):
                    w_copy(s + 1, lt).start()
            for lt in range(4):
                w_copy(s, lt).wait()
            def wbody(u, c, s=s):
                w_unit(s, u // 4, u % 4)
                return c
            lax.fori_loop(0, 8, wbody, 0)
        zd = jnp.zeros((_M, 128), jnp.bfloat16)
        for slot in range(2):
            for kt in range(8):
                dc[slot, 45, kt] = zd

    @pl.when(t + 1 < NQ)
    def _():
        x_start(t + 1)

    @pl.when(t < NQ)
    def _():
        x_wait(t)

    @pl.when(t == _NC + 2)
    def _():
        stats(0)

    @pl.when(t == 2 * _NC + 2)
    def _():
        stats(1)

    @pl.when(t == 0)
    def _():
        step(True, False, False, False)

    @pl.when(t == 1)
    def _():
        step(True, True, False, False)

    @pl.when(jnp.logical_and(t >= 2, t < _NC + 2))
    def _():
        step(True, True, True, False)

    @pl.when(jnp.logical_and(t >= _NC + 2, t < NQ))
    def _():
        step(True, True, True, True)

    @pl.when(t == NQ)
    def _():
        step(False, True, True, True)

    @pl.when(t == NQ + 1)
    def _():
        step(False, False, True, True)

    @pl.when(t >= NQ + 2)
    def _():
        step(False, False, False, True)


@jax.jit
def pallas_standalone__self_sup_conv_stem_wavlm__speech_kernel(x, w, gn_gamma, gn_beta):
    B, T, D = x.shape
    K = w.shape[0]
    L = (T - K) // 2 + 1
    assert (B, T, D, K) == (2, 16000, 512, 31)
    nsteps = 3 * _NC + 2

    def out_map(t):
        return (jnp.clip(t - (2 * _NC + 2), 0, _NC - 1), 0, 0)

    out = pl.pallas_call(
        functools.partial(_kernel, B=B, T=T, L=L),
        grid=(nsteps,),
        in_specs=[
            pl.BlockSpec(memory_space=pl.ANY),
            pl.BlockSpec(memory_space=pl.ANY),
            pl.BlockSpec((1, D), lambda t: (0, 0)),
            pl.BlockSpec((1, D), lambda t: (0, 0)),
        ],
        out_specs=pl.BlockSpec((_CR, B, D), out_map),
        out_shape=jax.ShapeDtypeStruct((L, B, D), jnp.bfloat16),
        scratch_shapes=[
            pltpu.VMEM((2, 4, 2 * _XW, 128), jnp.bfloat16),
            pltpu.VMEM((2, 4, K, 32, 128), jnp.bfloat16),
            pltpu.VMEM((_NP, 4, 2 * D, 128), jnp.bfloat16),
            pltpu.VMEM((2, _NP, 8, _M, 128), jnp.bfloat16),
            pltpu.VMEM((2, 32, 4, _M, 128), jnp.float32),
            pltpu.VMEM((B, 4, _HR, 128), jnp.float32),
            pltpu.VMEM((B, 2, 4, 8, 128), jnp.float32),
            pltpu.VMEM((2, 4, 8, 128), jnp.float32),
            pltpu.SemaphoreType.DMA((2,)),
            pltpu.SemaphoreType.DMA((2,)),
        ],
        compiler_params=pltpu.CompilerParams(
            dimension_semantics=("arbitrary",),
            vmem_limit_bytes=127 * 1024 * 1024,
        ),
    )(x, w, gn_gamma.reshape(1, D), gn_beta.reshape(1, D))
    return jnp.transpose(out, (1, 0, 2))
```

```python
import math
import functools
import jax
import jax.numpy as jnp
from jax import lax
from jax.experimental import pallas as pl
from jax.experimental.pallas import tpu as pltpu

class _Node:
    __slots__ = ("op", "args", "c", "idx")

class _Prog:
    def __init__(self):
        self.nodes = []
        self.cse = {}

    def _mk(self, op, args=(), c=None):
        key = (op, tuple(a.idx for a in args), c)
        n = self.cse.get(key)
        if n is None:
            n = _Node()
            n.op, n.args, n.c, n.idx = op, args, c, len(self.nodes)
            self.nodes.append(n)
            self.cse[key] = n
        return n

    def inp(self, i):
        return (1, self._mk("in", (), i))

    def neg(self, a):
        return None if a is None else (-a[0], a[1])

    def add(self, a, b):
        if a is None:
            return b
        if b is None:
            return a
        (sa, na), (sb, nb) = a, b
        if sa == sb:
            if na is nb:
                return (sa, self._mk("mul", (na,), 2.0))
            x, y = sorted((na, nb), key=lambda n: n.idx)
            return (sa, self._mk("add", (x, y)))
        if na is nb:
            return None
        if sa > 0:
            return (1, self._mk("sub", (na, nb)))
        return (1, self._mk("sub", (nb, na)))

    def sub(self, a, b):
        return self.add(a, self.neg(b))

    def mul(self, a, c):
        if a is None or abs(c) < 1e-12:
            return None
        if abs(c - 1) < 1e-12:
            return a
        if abs(c + 1) < 1e-12:
            return self.neg(a)
        return (a[0] * (1 if c > 0 else -1), self._mk("mul", (a[1],), abs(float(c))))


def _cadd(B, a, b): return (B.add(a[0], b[0]), B.add(a[1], b[1]))
def _csub(B, a, b): return (B.sub(a[0], b[0]), B.sub(a[1], b[1]))
def _cconj(B, a): return (a[0], B.neg(a[1]))
def _cmuli(B, a): return (B.neg(a[1]), a[0])
def _cmulni(B, a): return (a[1], B.neg(a[0]))


def _ctw(B, a, k, n):
    k %= n
    if k == 0:
        return a
    if 2 * k == n:
        return (B.neg(a[0]), B.neg(a[1]))
    if 4 * k == n:
        return _cmulni(B, a)
    if 4 * k == 3 * n:
        return _cmuli(B, a)
    th = -2 * math.pi * k / n
    c, s = math.cos(th), math.sin(th)
    if (8 * k) % n == 0:
        m = abs(c)
        f = lambda v, sg: v if sg > 0 else B.neg(v)
        re = B.sub(f(a[0], c), f(a[1], s))
        im = B.add(f(a[1], c), f(a[0], s))
        return (B.mul(re, m), B.mul(im, m))
    return (B.sub(B.mul(a[0], c), B.mul(a[1], s)), B.add(B.mul(a[1], c), B.mul(a[0], s)))


NF = 32


def _rdft(B, x):
    n = len(x)
    if n == 1:
        return [(x[0], None)]
    if n == 2:
        return [(B.add(x[0], x[1]), None), (B.sub(x[0], x[1]), None)]
    E = _rdft(B, x[0::2]); O1 = _rdft(B, x[1::4]); O3 = _rdft(B, x[3::4])
    if n == NF:
        cut = {}
        for grp in (O1, O3, E):
            for z in grp:
                for term in z:
                    if term is not None and term[1].op != "in":
                        cut[term[1].idx] = term[1]
        B.cut = cut
    X = [None] * n
    q = n // 4
    for k in range(0, q // 2 + 1):
        if k >= q:
            break
        a = _ctw(B, O1[k], k, n); b = _ctw(B, O3[k], 3 * k, n)
        s = _cadd(B, a, b); d = _cmuli(B, _csub(B, a, b))
        X[k] = _cadd(B, E[k], s)
        X[k + 2 * q] = _csub(B, E[k], s)
        X[k + q] = _csub(B, E[k + q], d)
        X[k + 3 * q] = _cadd(B, E[k + q], d)
    for k in range(n):
        if X[k] is None:
            X[k] = _cconj(B, X[n - k])
    return X


def _spectrum(B, x):
    X = _rdft(B, x)
    o = []
    for k in range(1, NF // 2):
        o += [X[k][0], X[k][1]]
    return o + [X[0][0], X[NF // 2][0]]


def data_program():
    B = _Prog()
    o = _spectrum(B, [B.inp(i) for i in range(NF)])
    outs = []
    for f in range(15):
        outs += [B.add(o[2 * f], o[2 * f + 1]), o[2 * f], o[2 * f + 1]]
    outs += [None, o[30], o[31]]
    return B, outs


def weight_program(ntaps):
    B = _Prog()
    o = _spectrum(B, [B.inp(i) if i < ntaps else None for i in range(NF)])
    outs = []
    for f in range(15):
        vr, vi = o[2 * f], B.neg(o[2 * f + 1])
        outs += [vr, B.sub(vi, vr), B.add(vr, vi)]
    outs += [None, B.mul(o[30], 0.5), B.mul(o[31], -0.5)]
    return B, outs


def output_program(nout):
    F = _Prog()
    o = _spectrum(F, [F.inp(i) if i < nout else None for i in range(NF)])
    B = _Prog()
    order = list(range(30)) + [31, 30]
    adj = {}
    def push(term, val):
        if term is None or val is None:
            return
        adj.setdefault(term[1].idx, []).append(val if term[0] > 0 else B.neg(val))
    for slot, k in enumerate(order):
        push(o[k], B.inp(slot))
    res = [None] * nout
    for n in reversed(F.nodes):
        terms = adj.get(n.idx)
        if not terms:
            continue
        a = terms[0]
        for t in terms[1:]:
            a = B.add(a, t)
        if n.op == "in":
            res[n.c] = a
        elif n.op == "add":
            push((1, n.args[0]), a); push((1, n.args[1]), a)
        elif n.op == "sub":
            push((1, n.args[0]), a); push((-1, n.args[1]), a)
        else:
            push((1, n.args[0]), B.mul(a, n.c))
    return B, res


def run_program(prog, inputs):
    B, outs = prog
    memo = {}
    get = inputs if callable(inputs) else inputs.__getitem__
    def ev(n):
        v = memo.get(n.idx)
        if v is None:
            if n.op == "in":
                v = get(n.c)
            elif n.op == "add":
                v = ev(n.args[0]) + ev(n.args[1])
            elif n.op == "sub":
                v = ev(n.args[0]) - ev(n.args[1])
            else:
                v = ev(n.args[0]) * n.c
            memo[n.idx] = v
        return v
    res = []
    for o in outs:
        if o is None:
            res.append(None)
        else:
            res.append((o[0], ev(o[1])))
    return res


def linearize(prog):
    B, outs = prog
    order, seen, where = [], set(), {}
    def visit(n):
        if n.idx in seen:
            return
        seen.add(n.idx)
        for a in n.args:
            visit(a)
        order.append(n)
    for k, o in enumerate(outs):
        if o is not None:
            visit(o[1])
            where.setdefault(o[1].idx, []).append((k, o[0]))
    return order, where


def gen_program(lin, ld, emit):
    order, where = lin
    vals = {}
    for n in order:
        if n.op == "in":
            v = ld(n.c)
        elif n.op == "add":
            v = vals[n.args[0].idx] + vals[n.args[1].idx]
        elif n.op == "sub":
            v = vals[n.args[0].idx] - vals[n.args[1].idx]
        else:
            v = vals[n.args[0].idx] * n.c
        vals[n.idx] = v
        for k, sg in where.get(n.idx, ()):
            emit(k, sg, v)
        yield 1


def staged(prog, groups):
    B, outs = prog
    need, seen = [], set()
    def visit(n):
        if n.idx in seen:
            return
        seen.add(n.idx)
        if n.idx in B.cut:
            need.append(n)
            return
        for a in n.args:
            visit(a)
    for grp in groups:
        for k in grp:
            if outs[k] is not None:
                visit(outs[k][1])
    need.sort(key=lambda n: n.idx)
    slot = {n.idx: q for q, n in enumerate(need)}
    lin1 = linearize((B, [(1, n) for n in need]))
    lin2 = []
    for grp in groups:
        order, where, seen2 = [], {}, set()
        def v2(n):
            if n.idx in seen2:
                return
            seen2.add(n.idx)
            if n.idx in slot:
                order.append(("ld", n))
                return
            for a in n.args:
                v2(a)
            order.append(("op", n))
        for k in grp:
            if outs[k] is not None:
                v2(outs[k][1])
                where.setdefault(outs[k][1].idx, []).append((k, outs[k][0]))
        lin2.append((order, where))
    return slot, lin1, lin2


def gen_stage2(lin2, slot, ld, emit):
    order, where = lin2
    vals = {}
    for kind, n in order:
        if kind == "ld":
            v = ld(slot[n.idx])
        elif n.op == "add":
            v = vals[n.args[0].idx] + vals[n.args[1].idx]
        elif n.op == "sub":
            v = vals[n.args[0].idx] - vals[n.args[1].idx]
        else:
            v = vals[n.args[0].idx] * n.c
        vals[n.idx] = v
        for k, sg in where.get(n.idx, ()):
            emit(k, sg, v)
        yield 1


def count_ops(prog):
    B, outs = prog
    seen = set(); st = [o[1] for o in outs if o is not None]; c = 0
    while st:
        n = st.pop()
        if n.idx in seen:
            continue
        seen.add(n.idx)
        c += n.op != "in"
        st.extend(n.args)
    return c


_DATA = data_program()
_WPROG = (weight_program(16), weight_program(15))
_S = 17
_OUT = output_program(_S)
_DLIN = linearize(_DATA)
_OLIN = linearize(_OUT)
_DGRP = [[3 * (fb - 1) + c for fb in grp for c in range(3)]
         for grp in ((1, 7, 9, 15), (2, 6, 10, 14), (3, 5, 11, 13), (4, 12, 8, 16))]
_DST = staged(_DATA, _DGRP)

_M = 96
_NC = 5
_CR = _M * _S
_HR = _NC * _CR
_XW = 1648
_NI = 8
_NP = 48


def _signed(t):
    return None if t is None else (t[1] if t[0] > 0 else -t[1])


def _kernel(x_hbm, w_hbm, g_ref, be_ref, o_ref,
            xs, wc, dc0, dc1, oc0, oc1, h0, h1, st, ab, tmp, xsem, wsem, *, B, T, L):
    dcs = (dc0, dc1); ocs = (oc0, oc1); hs = (h0, h1)
    t = pl.program_id(0)
    NQ = B * _NC
    xw = xs.bitcast(jnp.uint32)

    def x_copy(q, lt, rows):
        slot = q % 2
        b = q // _NC
        c = q % _NC
        r0 = pl.multiple_of(c * (2 * _CR), 16)
        return pltpu.make_async_copy(
            x_hbm.at[b, pl.ds(r0, rows), pl.ds(lt * 128, 128)],
            xs.at[slot, lt, pl.ds(0, rows)], xsem.at[slot])

    last_rows = T - (_NC - 1) * 2 * _CR

    def x_start(q):
        is_last = (q % _NC) == _NC - 1
        @pl.when(is_last)
        def _():
            for lt in range(4):
                x_copy(q, lt, last_rows).start()
            z = jnp.zeros((2 * _XW - last_rows, 128), jnp.bfloat16)
            for lt in range(4):
                xs[q % 2, lt, pl.ds(last_rows, 2 * _XW - last_rows), :] = z
        @pl.when(jnp.logical_not(is_last))
        def _():
            for lt in range(4):
                x_copy(q, lt, 2 * _XW).start()

    def x_wait(q):
        is_last = (q % _NC) == _NC - 1
        @pl.when(is_last)
        def _():
            for lt in range(4):
                x_copy(q, lt, last_rows).wait()
            lw = last_rows // 2
            for lt in range(4):
                v = xw[q % 2, lt, pl.ds(lw - 8, 8), :]
                row = lax.broadcasted_iota(jnp.int32, (8, 128), 0)
                xw[q % 2, lt, pl.ds(lw - 8, 8), :] = jnp.where(row == 7, v & jnp.uint32(0xFFFF), v)
        @pl.when(jnp.logical_not(is_last))
        def _():
            for lt in range(4):
                x_copy(q, lt, 2 * _XW).wait()

    def w_copy(s, lt):
        return pltpu.make_async_copy(
            w_hbm.bitcast(jnp.uint32).at[:, pl.ds(s * 16, 16), pl.ds(lt * 128, 128)],
            dc1.at[pl.ds(0, 31), (s % 2) * 4 + lt, pl.ds(0, 16)], wsem.at[s % 2])


    def w_unit(s, rg, lt):
        for ph in range(2):
            prog = _WPROG[ph]
            halves = []
            for hf in range(2):
                def ld(j):
                    wv = dc1[2 * j + ph, (s % 2) * 4 + lt, pl.ds(pl.multiple_of(rg * 8, 8), 8), :]
                    wv = (wv << 16) if hf == 0 else (wv & jnp.uint32(0xFFFF0000))
                    return pltpu.bitcast(wv, jnp.float32)
                halves.append(run_program(prog, ld))
            r0 = pl.multiple_of(ph * 256 + s * 16 + rg * 8, 8)
            for p, dv in enumerate(_DATA[1]):
                if halves[0][p] is None:
                    continue
                sg = halves[0][p][0] * dv[0]
                va, vb = halves[0][p][1], halves[1][p][1]
                if sg < 0:
                    va, vb = -va, -vb
                wc[p, lt, pl.ds(r0, 8), :] = pltpu.pack_elementwise([va, vb], packed_dtype=jnp.bfloat16)

    def d_unit(par, g, lt, ph):
        sub = xw.at[par, lt, pl.ds(pl.multiple_of(g * (16 * _S), 16), 288)]
        slot, lin1, lin2 = _DST
        tm = tmp.at[t // 64]
        for hf in range(2):
            def ld(j, hf=hf):
                w = sub[pl.ds(hf * _S + j, 8, stride=2 * _S), :]
                w = (w << 16) if ph == 0 else (w & jnp.uint32(0xFFFF0000))
                return pltpu.bitcast(w, jnp.float32)
            def emit(q, sg, v, hf=hf):
                tm[hf, q] = v
            yield from gen_program(lin1, ld, emit)
        for l2 in lin2:
            first = {}
            for hf in range(2):
                def emit(p, sg, v, hf=hf):
                    if hf == 0:
                        first[p] = v
                    else:
                        dcs[par][p, ph * 4 + lt, pl.ds(pl.multiple_of(g * 8, 8), 8), :] = pltpu.pack_elementwise(
                            [first[p], v], packed_dtype=jnp.bfloat16)
                yield from gen_stage2(l2, slot, lambda q, hf=hf: tm[hf, q], emit)

    def m_bin(slot, f):
        dc = dcs[slot]; oc = ocs[slot]
        for lt in range(4):
            k = []
            for c in range(3):
                p = 3 * f + c
                acc = None
                for kt in range(8):
                    lhs = pltpu.bitcast(dc[p, kt], jnp.bfloat16)
                    rhs = pltpu.bitcast(wc[p, lt, kt * 64:(kt + 1) * 64, :], jnp.bfloat16)
                    r = jnp.dot(lhs, rhs, preferred_element_type=jnp.float32)
                    acc = r if acc is None else acc + r
                    yield acc
                k.append(acc)
            oc[2 * f, lt, pl.ds(0, _M), :] = k[0] - k[2]
            oc[2 * f + 1, lt, pl.ds(0, _M), :] = k[0] + k[1]

    def o_unit(slot, b, c, g8, lt):
        oc = ocs[slot]
        ld = lambda k: oc[k, lt, pl.ds(pl.multiple_of(g8 * 8, 8), 8), :]
        blk0 = c * _M + g8 * 8
        sub = hs[b].at[lt, pl.ds(pl.multiple_of(blk0 * _S, 8), 8 * _S)]
        blk = blk0 + lax.broadcasted_iota(jnp.int32, (8, 128), 0)
        nfull = L // _S
        jr = L - nfull * _S
        m_lo = jnp.where(blk <= nfull, 1.0, 0.0).astype(jnp.float32)
        m_hi = jnp.where(blk < nfull, 1.0, 0.0).astype(jnp.float32)
        acc = [None, None]
        def emit(j, sg, v):
            y = v if sg > 0 else -v
            sub[pl.ds(j, 8, stride=_S), :] = y
            ym = y * (m_lo if j < jr else m_hi)
            acc[0] = ym if acc[0] is None else acc[0] + ym
            acc[1] = ym * ym if acc[1] is None else acc[1] + ym * ym
        yield from gen_program(_OLIN, ld, emit)
        st[b, 0, lt] += acc[0]
        st[b, 1, lt] += acc[1]

    def stats(b):
        for lt in range(4):
            s = jnp.sum(st[b, 0, lt], axis=0, keepdims=True) * (1.0 / L)
            q = jnp.sum(st[b, 1, lt], axis=0, keepdims=True) * (1.0 / L)
            var = jnp.maximum(q - s * s, 0.0) * (1.0 / 256.0)
            a = lax.rsqrt(var + 1e-5) * (1.0 / 16.0) * g_ref[:, lt * 128:(lt + 1) * 128].astype(jnp.float32)
            bb = be_ref[:, lt * 128:(lt + 1) * 128].astype(jnp.float32) - s * a
            ab[0, lt] = jnp.broadcast_to(a, (8, 128))
            ab[1, lt] = jnp.broadcast_to(bb, (8, 128))

    ou = o_ref.bitcast(jnp.uint32)

    def gelu_norm(b, lt, rows):
        z = hs[b][lt, rows, :] * ab[0, lt] + ab[1, lt]
        u = z * (0.7978845608028654 + 0.035677408136300125 * (z * z))
        return (0.5 * z) * (1.0 + jnp.tanh(u))

    def e_part(final, c, i):
        if not final:
            lt = i % 4
            for r in range(102):
                rows = pl.ds(pl.multiple_of(c * _CR + ((i // 4) * 102 + r) * 8, 8), 8)
                h0[lt, rows, :] = gelu_norm(0, lt, rows)
                yield 12
            return
        g0 = jnp.minimum(26 * i, _CR // 8 - 26)
        for r in range(26):
            rl = pl.multiple_of((g0 + r) * 8, 8)
            rows = pl.ds(pl.multiple_of(c * _CR + rl, 8), 8)
            if True:
                wv = [pltpu.pack_elementwise([h0[lt, rows, :], gelu_norm(1, lt, rows)],
                                             packed_dtype=jnp.bfloat16) for lt in range(4)]
                ou[pl.ds(rl, 8), 0, :] = jnp.concatenate(wv, axis=1)
                yield 48

    FILL = 0.95
    PINEVERY = 1
    PINROW = 0

    def step(par, D, Mm, O, E, ob=0):
        def body(i, carry):
            lt = i % 4
            hi = i // 4
            def chain(gens):
                for g_ in gens:
                    yield from g_
            vec = []
            nvec = 0
            if D:
                vec.append(chain(d_unit(par, hi * 3 + k // 2, lt, k % 2) for k in range(6)))
                nvec += 6 * 2 * len(_DLIN[0])
            if O:
                vec.append(chain(o_unit(par, ob, t - 2 - ob * _NC, hi * 6 + k, lt) for k in range(6)))
                nvec += 6 * len(_OLIN[0])
            if E:
                vec.append(e_part(not (D or Mm or O), ec, i))
                nvec += 102 * 12
            if Mm:
                tot = [6 * 2 * len(_DLIN[0]) if D else 0, 6 * len(_OLIN[0]) if O else 0, 102 * 12 if E else 0]
                tot = [v for v in tot if v]
                done = [0] * len(vec)
                alive = [True] * len(vec)
                nm = 192
                for step_i, accv in enumerate(chain(m_bin(1 - par, 2 * i + k) for k in range(2))):
                    if step_i % PINEVERY == PINEVERY - 1:
                        pv = accv[PINROW:PINROW + 8]
                        if D:
                            xw[par, lt, pl.ds(_XW, 8), :] = pltpu.bitcast(pv, jnp.uint32)
                            tmp[t // 64, 0, 32] = pv
                        if O:
                            ocs[par][31, lt, pl.ds(_M, 8), :] = pv
                        if E:
                            h0[lt, pl.ds(_HR, 8), :] = pv
                    frac = min(1.0, (step_i + 1) / (nm * FILL))
                    for q, g_ in enumerate(vec):
                        while alive[q] and done[q] < frac * tot[q]:
                            try:
                                done[q] += next(g_)
                            except StopIteration:
                                alive[q] = False
            for g_ in vec:
                for _ in g_:
                    pass
            return carry
        lax.fori_loop(0, _NI, body, 0)

    ec = jnp.where(t < 2 * _NC + 2, t - (_NC + 2), t - (2 * _NC + 2))

    @pl.when(t == 0)
    def _():
        x_start(0)
        for lt in range(4):
            w_copy(0, lt).start()
        st[...] = jnp.zeros(st.shape, jnp.float32)
        zc = jnp.zeros((512, 128), jnp.uint32)
        for lt in range(4):
            wc[45, lt] = zc
        def slab(s, c):
            @pl.when(s + 1 < 16)
            def _():
                for lt in range(4):
                    w_copy(s + 1, lt).start()
            for lt in range(4):
                w_copy(s, lt).wait()
            def wbody(u, c2):
                w_unit(s, u // 4, u % 4)
                return c2
            lax.fori_loop(0, 8, wbody, 0)
            return c
        lax.fori_loop(0, 16, slab, 0)
        zd = jnp.zeros((_M // 2, 128), jnp.uint32)
        for dc in dcs:
            for kt in range(8):
                dc[45, kt] = zd

    @pl.when(t + 1 < NQ)
    def _():
        x_start(t + 1)

    @pl.when(t < NQ)
    def _():
        x_wait(t)

    @pl.when(t == _NC + 2)
    def _():
        stats(0)

    @pl.when(t == 2 * _NC + 2)
    def _():
        stats(1)

    def both(cond, *flags, **kw):
        for par in range(2):
            @pl.when(jnp.logical_and(cond, t % 2 == par))
            def _():
                step(par, *flags, **kw)

    pl.when(t == 0)(lambda: step(0, True, False, False, False))
    pl.when(t == 1)(lambda: step(1, True, True, False, False))
    both(jnp.logical_and(t >= 2, t < _NC + 2), True, True, True, False, ob=0)
    both(jnp.logical_and(t >= _NC + 2, t < NQ), True, True, True, True, ob=1)
    pl.when(t == NQ)(lambda: step(NQ % 2, False, True, True, True, ob=1))
    pl.when(t == NQ + 1)(lambda: step((NQ + 1) % 2, False, False, True, True, ob=1))
    pl.when(t >= NQ + 2)(lambda: step(0, False, False, False, True))


@jax.jit
def pallas_standalone__self_sup_conv_stem_wavlm__speech_kernel(x, w, gn_gamma, gn_beta):
    B, T, D = x.shape
    K = w.shape[0]
    L = (T - K) // 2 + 1
    assert (B, T, D, K) == (2, 16000, 512, 31)
    nsteps = 3 * _NC + 2

    def out_map(t):
        return (jnp.clip(t - (2 * _NC + 2), 0, _NC - 1), 0, 0)

    out = pl.pallas_call(
        functools.partial(_kernel, B=B, T=T, L=L),
        grid=(nsteps,),
        in_specs=[
            pl.BlockSpec(memory_space=pl.ANY),
            pl.BlockSpec(memory_space=pl.ANY),
            pl.BlockSpec((1, D), lambda t: (0, 0)),
            pl.BlockSpec((1, D), lambda t: (0, 0)),
        ],
        out_specs=pl.BlockSpec((_CR, B, D), out_map),
        out_shape=jax.ShapeDtypeStruct((L, B, D), jnp.bfloat16),
        scratch_shapes=[
            pltpu.VMEM((2, 4, 2 * _XW + 16, 128), jnp.bfloat16),
            pltpu.VMEM((_NP, 4, D, 128), jnp.uint32),
            pltpu.VMEM((_NP, 8, _M // 2, 128), jnp.uint32),
            pltpu.VMEM((_NP, 8, _M // 2, 128), jnp.uint32),
            pltpu.VMEM((32, 4, _M + 8, 128), jnp.float32),
            pltpu.VMEM((32, 4, _M + 8, 128), jnp.float32),
            pltpu.VMEM((4, _HR + 8, 128), jnp.float32),
            pltpu.VMEM((4, _HR, 128), jnp.float32),
            pltpu.VMEM((B, 2, 4, 8, 128), jnp.float32),
            pltpu.VMEM((2, 4, 8, 128), jnp.float32),
            pltpu.VMEM((1, 2, 33, 8, 128), jnp.float32),
            pltpu.SemaphoreType.DMA((2,)),
            pltpu.SemaphoreType.DMA((2,)),
        ],
        compiler_params=pltpu.CompilerParams(
            dimension_semantics=("arbitrary",),
            vmem_limit_bytes=127 * 1024 * 1024,
        ),
    )(x, w, gn_gamma.reshape(1, D), gn_beta.reshape(1, D))
    return jnp.transpose(out, (1, 0, 2))
```

```python
import math
import functools
import jax
import jax.numpy as jnp
from jax import lax
from jax.experimental import pallas as pl
from jax.experimental.pallas import tpu as pltpu

NF = 40


class _Node:
    __slots__ = ("op", "args", "c", "idx")


class _Prog:
    def __init__(self):
        self.nodes = []
        self.cse = {}
        self.cut = {}

    def _mk(self, op, args=(), c=None):
        key = (op, tuple(a.idx for a in args), c)
        n = self.cse.get(key)
        if n is None:
            n = _Node()
            n.op, n.args, n.c, n.idx = op, args, c, len(self.nodes)
            self.nodes.append(n)
            self.cse[key] = n
        return n

    def inp(self, i):
        return (1, self._mk("in", (), i))

    def neg(self, a):
        return None if a is None else (-a[0], a[1])

    def add(self, a, b):
        if a is None:
            return b
        if b is None:
            return a
        (sa, na), (sb, nb) = a, b
        if sa == sb:
            if na is nb:
                return (sa, self._mk("mul", (na,), 2.0))
            x, y = sorted((na, nb), key=lambda n: n.idx)
            return (sa, self._mk("add", (x, y)))
        if na is nb:
            return None
        if sa > 0:
            return (1, self._mk("sub", (na, nb)))
        return (1, self._mk("sub", (nb, na)))

    def sub(self, a, b):
        return self.add(a, self.neg(b))

    def mul(self, a, c):
        if a is None or abs(c) < 1e-12:
            return None
        if abs(c - 1) < 1e-12:
            return a
        if abs(c + 1) < 1e-12:
            return self.neg(a)
        return (a[0] * (1 if c > 0 else -1), self._mk("mul", (a[1],), abs(float(c))))


def _cadd(B, a, b): return (B.add(a[0], b[0]), B.add(a[1], b[1]))
def _csub(B, a, b): return (B.sub(a[0], b[0]), B.sub(a[1], b[1]))
def _cscale(B, a, c): return (B.mul(a[0], c), B.mul(a[1], c))
def _cconj(B, a): return (a[0], B.neg(a[1]))
def _cmuli(B, a): return (B.neg(a[1]), a[0])


def _rdft8(B, x):
    a0, a1 = B.add(x[0], x[4]), B.sub(x[0], x[4])
    b0, b1 = B.add(x[2], x[6]), B.sub(x[2], x[6])
    c0, c1 = B.add(x[1], x[5]), B.sub(x[1], x[5])
    d0, d1 = B.add(x[3], x[7]), B.sub(x[3], x[7])
    e0, e2 = B.add(a0, b0), B.sub(a0, b0)
    o0, o2 = B.add(c0, d0), B.sub(c0, d0)
    r = math.sqrt(0.5)
    p = B.mul(B.sub(c1, d1), r)
    q = B.mul(B.add(c1, d1), r)
    return [
        (B.add(e0, o0), None),
        (B.add(a1, p), B.neg(B.add(b1, q))),
        (e2, B.neg(o2)),
        (B.sub(a1, p), B.sub(b1, q)),
        (B.sub(e0, o0), None),
    ]


def _cdft5(B, z):
    t1, t2 = _cadd(B, z[1], z[4]), _cadd(B, z[2], z[3])
    t3, t4 = _csub(B, z[1], z[4]), _csub(B, z[2], z[3])
    m = _cadd(B, t1, t2)
    x0 = _cadd(B, z[0], m)
    u = _csub(B, z[0], _cscale(B, m, 0.25))
    v = _cscale(B, _csub(B, t1, t2), math.sqrt(5.0) / 4.0)
    a1, a2 = _cadd(B, u, v), _csub(B, u, v)
    s1, s2 = math.sin(2 * math.pi / 5), math.sin(4 * math.pi / 5)
    b1 = _cadd(B, _cscale(B, t3, s1), _cscale(B, t4, s2))
    b2 = _csub(B, _cscale(B, t3, s2), _cscale(B, t4, s1))
    ib1, ib2 = _cmuli(B, b1), _cmuli(B, b2)
    return [x0, _csub(B, a1, ib1), _csub(B, a2, ib2), _cadd(B, a2, ib2), _cadd(B, a1, ib1)]


_BINS = [(k2, k1) for k2 in (1, 2, 3) for k1 in range(5)] + [(0, 1), (0, 2), (4, 1), (4, 2)]
_NCB = len(_BINS)


def _spectrum(B, x):
    z = [_rdft8(B, [x[(8 * n1 + 5 * n2) % NF] for n2 in range(8)]) for n1 in range(5)]
    for row in z:
        for c in row:
            for term in c:
                if term is not None and term[1].op != "in":
                    B.cut[term[1].idx] = term[1]
    X = [_cdft5(B, [z[n1][k2] for n1 in range(5)]) for k2 in range(5)]
    o = []
    for k2, k1 in _BINS:
        o += [X[k2][k1][0], X[k2][k1][1]]
    return o + [X[0][0][0], X[4][0][0]]


def data_program():
    B = _Prog()
    o = _spectrum(B, [B.inp(i) for i in range(NF)])
    outs = []
    for f in range(_NCB):
        outs += [B.add(o[2 * f], o[2 * f + 1]), o[2 * f], o[2 * f + 1]]
    outs += [None, o[2 * _NCB], o[2 * _NCB + 1]]
    return B, outs


def weight_program(ntaps):
    B = _Prog()
    o = _spectrum(B, [B.inp(i) if i < ntaps else None for i in range(NF)])
    outs = []
    for f in range(_NCB):
        vr, vi = o[2 * f], B.neg(o[2 * f + 1])
        outs += [vr, B.sub(vi, vr), B.add(vr, vi)]
    outs += [None, B.mul(o[2 * _NCB], 0.5), B.mul(o[2 * _NCB + 1], -0.5)]
    return B, outs


def output_program(nout):
    F = _Prog()
    o = _spectrum(F, [F.inp(i) if i < nout else None for i in range(NF)])
    B = _Prog()
    order = list(range(2 * _NCB)) + [2 * _NCB + 1, 2 * _NCB]
    adj = {}

    def push(term, val):
        if term is None or val is None:
            return
        adj.setdefault(term[1].idx, []).append(val if term[0] > 0 else B.neg(val))

    for slot, k in enumerate(order):
        push(o[k], B.inp(slot))
    res = [None] * nout
    for n in reversed(F.nodes):
        terms = adj.get(n.idx)
        if not terms:
            continue
        a = terms[0]
        for t in terms[1:]:
            a = B.add(a, t)
        if n.idx in F.cut and a[1].op != "in":
            B.cut[a[1].idx] = a[1]
        if n.op == "in":
            res[n.c] = a
        elif n.op == "add":
            push((1, n.args[0]), a); push((1, n.args[1]), a)
        elif n.op == "sub":
            push((1, n.args[0]), a); push((-1, n.args[1]), a)
        else:
            push((1, n.args[0]), B.mul(a, n.c))
    return B, res


def linearize(prog):
    B, outs = prog
    order, seen, where = [], set(), {}

    def visit(n):
        if n.idx in seen:
            return
        seen.add(n.idx)
        for a in n.args:
            visit(a)
        order.append(n)

    for k, o in enumerate(outs):
        if o is not None:
            visit(o[1])
            where.setdefault(o[1].idx, []).append((k, o[0]))
    return order, where


def staged(prog, groups):
    B, outs = prog
    need, seen = [], set()

    def visit(n):
        if n.idx in seen:
            return
        seen.add(n.idx)
        if n.idx in B.cut or n.op == "in":
            need.append(n)
            return
        for a in n.args:
            visit(a)

    for grp in groups:
        for k in grp:
            if outs[k] is not None:
                visit(outs[k][1])
    need.sort(key=lambda n: n.idx)
    slot = {n.idx: q for q, n in enumerate(need)}
    lin1 = linearize((B, [(1, n) for n in need]))
    lin2 = []
    for grp in groups:
        order, where, seen2 = [], {}, set()

        def v2(n):
            if n.idx in seen2:
                return
            seen2.add(n.idx)
            if n.idx in slot:
                order.append(("ld", n))
                return
            for a in n.args:
                v2(a)
            order.append(("op", n))

        for k in grp:
            if outs[k] is not None:
                v2(outs[k][1])
                where.setdefault(outs[k][1].idx, []).append((k, outs[k][0]))
        lin2.append((order, where))
    return slot, lin1, lin2


def _apply(n, vals):
    if n.op == "add":
        return vals[n.args[0].idx] + vals[n.args[1].idx]
    if n.op == "sub":
        return vals[n.args[0].idx] - vals[n.args[1].idx]
    return vals[n.args[0].idx] * n.c


def gen_program(lin, ld, emit):
    order, where = lin
    vals = {}
    for n in order:
        v = ld(n.c) if n.op == "in" else _apply(n, vals)
        vals[n.idx] = v
        for k, sg in where.get(n.idx, ()):
            emit(k, sg, v)
        yield 1


def gen_stage2(lin2, slot, ld, emit):
    order, where = lin2
    vals = {}
    for kind, n in order:
        v = ld(slot[n.idx]) if kind == "ld" else _apply(n, vals)
        vals[n.idx] = v
        for k, sg in where.get(n.idx, ()):
            emit(k, sg, v)
        yield 1


_S = 25
_M = 64
_NC = 5
_CR = _M * _S
_HR = _NC * _CR
_XW = 1616
_NS = 20
_NP = 3 * _NS
_SCALE = NF / 2

_DATA = data_program()
_OUT = output_program(_S)
_GRP = [[3 * f + c for f in range(5 * g, 5 * g + 5) for c in range(3)] for g in range(4)]
_DST = staged(_DATA, _GRP)
_WST = (staged(weight_program(16), _GRP), staged(weight_program(15), _GRP))
_OLIN = linearize(_OUT)
_DOPS = 2 * (len(_DST[1][0]) + sum(len(l[0]) for l in _DST[2]))
_WOPS = sum(2 * (len(w[1][0]) + sum(len(l[0]) for l in w[2])) for w in _WST)
_OOPS = len(_OLIN[0])


def _chain(gens):
    for g in gens:
        yield from g


def _kernel(x_hbm, w_hbm, g_ref, be_ref, o_hbm,
            xs, wc0, wc1, wc2, wc3, dc0, dc1, oc0, oc1, h0, h1, st, ab, tmp, xsem, wsem, osem, *, B, T, L):
    wcs = (wc0, wc1, wc2, wc3)
    dcs = (dc0, dc1); ocs = (oc0, oc1); hs = (h0, h1)
    NQ = B * _NC
    xw = xs.bitcast(jnp.uint32)
    h1u = h1.bitcast(jnp.uint32)
    ou = o_hbm.bitcast(jnp.uint32)
    wu = w_hbm.bitcast(jnp.uint32)
    zbox = [0]

    last_rows = T - (_NC - 1) * 2 * _CR
    full_rows = 2 * _XW

    def x_copy(q, par, lt, rows):
        b = q // _NC
        r0 = pl.multiple_of((q % _NC) * (2 * _CR), 16)
        return pltpu.make_async_copy(
            x_hbm.at[b, pl.ds(r0, rows), pl.ds(lt * 128, 128)],
            xs.at[par, lt, pl.ds(0, rows)], xsem.at[par])

    def x_start(q, par, last):
        for lt in range(4):
            x_copy(q, par, lt, last_rows if last else full_rows).start()
        if last:
            z = jnp.zeros((full_rows - last_rows, 128), jnp.bfloat16)
            for lt in range(4):
                xs[par, lt, pl.ds(last_rows, full_rows - last_rows), :] = z

    def x_wait(q, par, last):
        for lt in range(4):
            x_copy(q, par, lt, last_rows if last else full_rows).wait()
        if last:
            lw = last_rows // 2
            row = lax.broadcasted_iota(jnp.int32, (8, 128), 0)
            for lt in range(4):
                v = xw[par, lt, pl.ds(lw - 8, 8), :]
                xw[par, lt, pl.ds(lw - 8, 8), :] = jnp.where(row == 7, v & jnp.uint32(0xFFFF), v)

    def w_copy(lt, tap):
        return pltpu.make_async_copy(wu.at[tap, :, pl.ds(lt * 128, 128)],
                                     h1u.at[lt, pl.ds(tap * 256, 256)], wsem.at[lt])

    def o_copy(c, lt):
        n = min(_CR, L - c * _CR)
        return pltpu.make_async_copy(h1u.at[lt, pl.ds(c * _CR, n)],
                                     ou.at[pl.ds(c * _CR, n), 0, pl.ds(lt * 128, 128)], osem.at[0])

    def staged_unit(prog, ld_word, split, put):
        slot, lin1, lin2 = prog
        tm = tmp.at[zbox[0]]
        for hf in range(2):
            def emit(q, sg, v, hf=hf):
                tm[hf, q] = v
            yield from gen_program(lin1, lambda j, hf=hf: ld_word(j, hf), emit)
        for l2 in lin2:
            first = {}
            for hf in range(2):
                def emit(p, sg, v, hf=hf):
                    if hf == 0:
                        first[p] = v
                    else:
                        a, b = first[p], v
                        if split(p) * sg < 0:
                            a, b = -a, -b
                        put(p, pltpu.pack_elementwise([a, b], packed_dtype=jnp.bfloat16))
                yield from gen_stage2(l2, slot, lambda q, hf=hf: tm[hf, q], emit)

    def w_unit(lt, u):
        for ph in range(2):
            def ld(j, hf, ph=ph):
                wv = h1u[lt, pl.ds(pl.multiple_of((2 * j + ph) * 256 + u * 8, 8), 8), :]
                wv = (wv << 16) if hf == 0 else (wv & jnp.uint32(0xFFFF0000))
                return pltpu.bitcast(wv, jnp.float32)
            def put(p, v, ph=ph):
                wcs[lt][p, pl.ds(pl.multiple_of(ph * 256 + u * 8, 8), 8), :] = v
            yield from staged_unit(_WST[ph], ld, lambda p: _DATA[1][p][0], put)

    def d_unit(par, g, lt, ph):
        sub = xw.at[par, lt, pl.ds(pl.multiple_of(g * (16 * _S), 16), 416)]
        def ld(j, hf):
            w = sub[pl.ds(hf * _S + j, 8, stride=2 * _S), :]
            w = (w << 16) if ph == 0 else (w & jnp.uint32(0xFFFF0000))
            return pltpu.bitcast(w, jnp.float32)
        def put(p, v):
            dcs[par][p, ph * 4 + lt, pl.ds(pl.multiple_of(g * 8, 8), 8), :] = v
        yield from staged_unit(_DST, ld, lambda p: _DATA[1][p][0], put)

    def o_unit(par, b, c, g8, lt):
        oc = ocs[par]
        ld = lambda k: oc[k, lt, pl.ds(pl.multiple_of(g8 * 8, 8), 8), :]
        blk0 = c * _M + g8 * 8
        sub = hs[b].at[lt, pl.ds(pl.multiple_of(blk0 * _S, 8), 8 * _S)]
        blk = blk0 + lax.broadcasted_iota(jnp.int32, (8, 128), 0)
        nfull = L // _S
        jr = L - nfull * _S
        m_lo = jnp.where(blk <= nfull, 1.0, 0.0).astype(jnp.float32)
        m_hi = jnp.where(blk < nfull, 1.0, 0.0).astype(jnp.float32)
        acc = [None, None]
        def emit(j, sg, v):
            y = v if sg > 0 else -v
            sub[pl.ds(j, 8, stride=_S), :] = y
            ym = y * (m_lo if j < jr else m_hi)
            acc[0] = ym if acc[0] is None else acc[0] + ym
            acc[1] = ym * ym if acc[1] is None else acc[1] + ym * ym
        yield from gen_program(_OLIN, ld, emit)
        st[b, 0, lt] += acc[0]
        st[b, 1, lt] += acc[1]

    def stats(b):
        for lt in range(4):
            s = jnp.sum(st[b, 0, lt], axis=0, keepdims=True) * (1.0 / L)
            q = jnp.sum(st[b, 1, lt], axis=0, keepdims=True) * (1.0 / L)
            var = jnp.maximum(q - s * s, 0.0) * (1.0 / (_SCALE * _SCALE))
            a = lax.rsqrt(var + 1e-5) * (1.0 / _SCALE) * g_ref[:, lt * 128:(lt + 1) * 128].astype(jnp.float32)
            bb = be_ref[:, lt * 128:(lt + 1) * 128].astype(jnp.float32) - s * a
            ab[0, lt] = jnp.broadcast_to(a, (8, 128))
            ab[1, lt] = jnp.broadcast_to(bb, (8, 128))

    def gelu_norm(b, lt, rows):
        z = hs[b][lt, rows, :] * ab[0, lt] + ab[1, lt]
        u = z * (0.7978845608028654 + 0.035677408136300125 * (z * z))
        return (0.5 * z) * (1.0 + jnp.tanh(u))

    def e_unit(final, c, lt):
        for r in range(_CR // 8):
            rows = pl.ds(pl.multiple_of(c * _CR + r * 8, 8), 8)
            if final:
                h1u[lt, rows, :] = pltpu.pack_elementwise(
                    [h0[lt, rows, :], gelu_norm(1, lt, rows)], packed_dtype=jnp.bfloat16)
            else:
                h0[lt, rows, :] = gelu_norm(0, lt, rows)
            yield 12

    def m_dots(par, slots, lts):
        dc = dcs[par]; oc = ocs[par]
        for f in slots:
            for lt in lts:
                k = []
                for c in range(3):
                    p = 3 * f + c
                    acc = None
                    for kt in range(8):
                        lhs = pltpu.bitcast(dc[p, kt], jnp.bfloat16)
                        rhs = pltpu.bitcast(wcs[lt][p, kt * 64:(kt + 1) * 64, :], jnp.bfloat16)
                        r = jnp.dot(lhs, rhs, preferred_element_type=jnp.float32)
                        acc = r if acc is None else acc + r
                        yield acc
                    k.append(acc)
                oc[2 * f, lt, pl.ds(0, _M), :] = k[0] - k[2]
                oc[2 * f + 1, lt, pl.ds(0, _M), :] = k[0] + k[1]

    FILL = 0.95

    def weave(mstream, nm, vec):
        done = [0] * len(vec)
        alive = [True] * len(vec)
        if mstream is not None:
            for k, acc in enumerate(mstream):
                pv = acc[0:8]
                frac = min(1.0, (k + 1) / (nm * FILL))
                for q, (g, tot, pin) in enumerate(vec):
                    if alive[q]:
                        pin(pv)
                    while alive[q] and done[q] < frac * tot:
                        try:
                            done[q] += next(g)
                        except StopIteration:
                            alive[q] = False
        for g, _, _ in vec:
            for _ in g:
                pass

    def pin_d(par, lt):
        def pin(v):
            xw[par, lt, pl.ds(pl.multiple_of(_XW + zbox[0], 8), 8), :] = pltpu.bitcast(v, jnp.uint32)
            tmp[zbox[0], 0, NF] = v
        return pin

    def pin_w(lt):
        def pin(v):
            h1[lt, pl.ds(pl.multiple_of(_HR + zbox[0], 8), 8), :] = v
            tmp[zbox[0], 0, NF] = v
        return pin

    def pin_o(par, lt):
        def pin(v):
            ocs[par][0, lt, pl.ds(pl.multiple_of(_M + zbox[0], 8), 8), :] = v
        return pin

    def pin_e(lt):
        def pin(v):
            h0[lt, pl.ds(pl.multiple_of(_HR + zbox[0], 8), 8), :] = v
        return pin

    def d_lt(par, lt):
        return (_chain(d_unit(par, k // 2, lt, k % 2) for k in range(8)), 8 * _DOPS, pin_d(par, lt))

    def o_lt(par, b, c, lt):
        return (_chain(o_unit(par, b, c, g8, lt) for g8 in range(8)), 8 * _OOPS, pin_o(par, lt))

    def e_lt(c, lt):
        return (e_unit(False, c, lt), 12 * (_CR // 8), pin_e(lt))

    def w_part(lt, u0, n):
        return (_chain(w_unit(lt, u0 + k) for k in range(n)), n * _WOPS, pin_w(lt))

    def step(t, par, D, Mm, O, E, ob):
        def body(i, carry):
            zbox[0] = i // 64
            vec = []
            if D:
                vec.append(d_lt(par, i))
            if O:
                vec.append(o_lt(par, ob, t - 2 - ob * _NC, i))
            if E:
                vec.append(e_lt(t - (_NC + 2), i))
            ms = m_dots(1 - par, [5 * i + k for k in range(5)], range(4)) if Mm else None
            weave(ms, 480, vec)
            return carry
        lax.fori_loop(0, 4, body, 0)

    for tap in range(31):
        w_copy(0, tap).start()
    x_start(0, 0, False)
    x_start(1, 1, False)
    for lt in range(1, 4):
        for tap in range(31):
            w_copy(lt, tap).start()
    st[...] = jnp.zeros(st.shape, jnp.float32)
    zc = jnp.zeros((512, 128), jnp.uint32)
    for lt in range(4):
        wcs[lt][_NP - 3] = zc
    zd = jnp.zeros((_M // 2, 128), jnp.uint32)
    for dc in dcs:
        for kt in range(8):
            dc[_NP - 3, kt] = zd

    def w_wait(lt):
        for tap in range(31):
            w_copy(lt, tap).wait()

    w_wait(0)
    def w0_body(u, c):
        zbox[0] = u // 64
        weave(None, 0, [w_part(0, 2 * u, 2)])
        return c
    lax.fori_loop(0, 16, w0_body, 0)
    for par in range(2):
        x_wait(par, par, False)
        def d0_body(i, c, par=par):
            zbox[0] = i // 64
            weave(None, 0, [d_lt(par, i)])
            return c
        lax.fori_loop(0, 4, d0_body, 0)

    for lt in range(3):
        w_wait(lt + 1)
        for par in range(2):
            def inner(k, c2, par=par, lt=lt):
                zbox[0] = k // 64
                weave(m_dots(par, [5 * k + j for j in range(5)], [lt]), 120,
                      [w_part(lt + 1, 16 * par + 4 * k, 4)])
                return c2
            lax.fori_loop(0, 4, inner, 0)

    x_start(2, 0, False)
    def last0(k, c):
        zbox[0] = k // 64
        weave(m_dots(0, [5 * k + j for j in range(5)], [3]), 120, [])
        return c
    lax.fori_loop(0, 4, last0, 0)
    x_wait(2, 0, False)
    x_start(3, 1, False)
    def last1(k, c):
        zbox[0] = k // 64
        weave(m_dots(1, [5 * k + j for j in range(5)], [3]), 120, [d_lt(0, k), o_lt(0, 0, 0, k)])
        return c
    lax.fori_loop(0, 4, last1, 0)

    def advance(t, par, last_now, last_next):
        x_wait(t, par, last_now)
        if last_next is not None:
            x_start(t + 1, 1 - par, last_next)

    def pair(k, c):
        t = 3 + 2 * k
        advance(t, 1, False, None)
        @pl.when(k == 0)
        def _():
            x_start(t + 1, 0, True)
        @pl.when(k != 0)
        def _():
            x_start(t + 1, 0, False)
        step(t, 1, True, True, True, False, 0)
        @pl.when(k == 0)
        def _():
            x_wait(t + 1, 0, True)
        @pl.when(k != 0)
        def _():
            x_wait(t + 1, 0, False)
        x_start(t + 2, 1, False)
        step(t + 1, 0, True, True, True, False, 0)
        return c
    lax.fori_loop(0, 2, pair, 0)
    stats(0)
    advance(7, 1, False, False)
    step(7, 1, True, True, True, True, 1)
    advance(8, 0, False, True)
    step(8, 0, True, True, True, True, 1)
    advance(9, 1, True, None)
    step(9, 1, True, True, True, True, 1)
    step(10, 0, False, True, True, True, 1)
    step(11, 1, False, False, True, True, 1)

    stats(1)

    def fin(k, c):
        return c
    for cch in range(_NC):
        def fbody(lt, c, cch=cch):
            for _ in e_unit(True, cch, lt):
                pass
            return c
        lax.fori_loop(0, 4, fbody, 0)
        for lt in range(4):
            o_copy(cch, lt).start()
    for cch in range(_NC):
        for lt in range(4):
            o_copy(cch, lt).wait()


@jax.jit
def pallas_standalone__self_sup_conv_stem_wavlm__speech_kernel(x, w, gn_gamma, gn_beta):
    B, T, D = x.shape
    K = w.shape[0]
    L = (T - K) // 2 + 1
    assert (B, T, D, K) == (2, 16000, 512, 31)
    out = pl.pallas_call(
        functools.partial(_kernel, B=B, T=T, L=L),
        grid=(1,),
        in_specs=[
            pl.BlockSpec(memory_space=pl.ANY),
            pl.BlockSpec(memory_space=pl.ANY),
            pl.BlockSpec((1, D), lambda t: (0, 0)),
            pl.BlockSpec((1, D), lambda t: (0, 0)),
        ],
        out_specs=pl.BlockSpec(memory_space=pl.ANY),
        out_shape=jax.ShapeDtypeStruct((L, B, D), jnp.bfloat16),
        scratch_shapes=[
            pltpu.VMEM((2, 4, 2 * _XW + 16, 128), jnp.bfloat16),
            *[pltpu.VMEM((_NP, D, 128), jnp.uint32) for _ in range(4)],
            pltpu.VMEM((_NP, 8, _M // 2, 128), jnp.uint32),
            pltpu.VMEM((_NP, 8, _M // 2, 128), jnp.uint32),
            pltpu.VMEM((NF, 4, _M + 8, 128), jnp.float32),
            pltpu.VMEM((NF, 4, _M + 8, 128), jnp.float32),
            pltpu.VMEM((4, _HR + 8, 128), jnp.float32),
            pltpu.VMEM((4, _HR + 8, 128), jnp.float32),
            pltpu.VMEM((B, 2, 4, 8, 128), jnp.float32),
            pltpu.VMEM((2, 4, 8, 128), jnp.float32),
            pltpu.VMEM((1, 2, NF + 1, 8, 128), jnp.float32),
            pltpu.SemaphoreType.DMA((2,)),
            pltpu.SemaphoreType.DMA((4,)),
            pltpu.SemaphoreType.DMA((1,)),
        ],
        compiler_params=pltpu.CompilerParams(
            dimension_semantics=("arbitrary",),
            vmem_limit_bytes=127 * 1024 * 1024,
        ),
    )(x, w, gn_gamma.reshape(1, D), gn_beta.reshape(1, D))
    return jnp.transpose(out, (1, 0, 2))
```

```python
import math
import functools
import jax
import jax.numpy as jnp
from jax import lax
from jax.experimental import pallas as pl
from jax.experimental.pallas import tpu as pltpu

NF = 40


class _Node:
    __slots__ = ("op", "args", "c", "idx")


class _Prog:
    def __init__(self):
        self.nodes = []
        self.cse = {}
        self.cut = {}

    def _mk(self, op, args=(), c=None):
        key = (op, tuple(a.idx for a in args), c)
        n = self.cse.get(key)
        if n is None:
            n = _Node()
            n.op, n.args, n.c, n.idx = op, args, c, len(self.nodes)
            self.nodes.append(n)
            self.cse[key] = n
        return n

    def inp(self, i):
        return (1, self._mk("in", (), i))

    def neg(self, a):
        return None if a is None else (-a[0], a[1])

    def add(self, a, b):
        if a is None:
            return b
        if b is None:
            return a
        (sa, na), (sb, nb) = a, b
        if sa == sb:
            if na is nb:
                return (sa, self._mk("mul", (na,), 2.0))
            x, y = sorted((na, nb), key=lambda n: n.idx)
            return (sa, self._mk("add", (x, y)))
        if na is nb:
            return None
        if sa > 0:
            return (1, self._mk("sub", (na, nb)))
        return (1, self._mk("sub", (nb, na)))

    def sub(self, a, b):
        return self.add(a, self.neg(b))

    def mul(self, a, c):
        if a is None or abs(c) < 1e-12:
            return None
        if abs(c - 1) < 1e-12:
            return a
        if abs(c + 1) < 1e-12:
            return self.neg(a)
        return (a[0] * (1 if c > 0 else -1), self._mk("mul", (a[1],), abs(float(c))))


def _cadd(B, a, b): return (B.add(a[0], b[0]), B.add(a[1], b[1]))
def _csub(B, a, b): return (B.sub(a[0], b[0]), B.sub(a[1], b[1]))
def _cscale(B, a, c): return (B.mul(a[0], c), B.mul(a[1], c))
def _cconj(B, a): return (a[0], B.neg(a[1]))
def _cmuli(B, a): return (B.neg(a[1]), a[0])


def _rdft8(B, x):
    a0, a1 = B.add(x[0], x[4]), B.sub(x[0], x[4])
    b0, b1 = B.add(x[2], x[6]), B.sub(x[2], x[6])
    c0, c1 = B.add(x[1], x[5]), B.sub(x[1], x[5])
    d0, d1 = B.add(x[3], x[7]), B.sub(x[3], x[7])
    e0, e2 = B.add(a0, b0), B.sub(a0, b0)
    o0, o2 = B.add(c0, d0), B.sub(c0, d0)
    r = math.sqrt(0.5)
    p = B.mul(B.sub(c1, d1), r)
    q = B.mul(B.add(c1, d1), r)
    return [
        (B.add(e0, o0), None),
        (B.add(a1, p), B.neg(B.add(b1, q))),
        (e2, B.neg(o2)),
        (B.sub(a1, p), B.sub(b1, q)),
        (B.sub(e0, o0), None),
    ]


def _cdft5(B, z):
    t1, t2 = _cadd(B, z[1], z[4]), _cadd(B, z[2], z[3])
    t3, t4 = _csub(B, z[1], z[4]), _csub(B, z[2], z[3])
    m = _cadd(B, t1, t2)
    x0 = _cadd(B, z[0], m)
    u = _csub(B, z[0], _cscale(B, m, 0.25))
    v = _cscale(B, _csub(B, t1, t2), math.sqrt(5.0) / 4.0)
    a1, a2 = _cadd(B, u, v), _csub(B, u, v)
    s1, s2 = math.sin(2 * math.pi / 5), math.sin(4 * math.pi / 5)
    b1 = _cadd(B, _cscale(B, t3, s1), _cscale(B, t4, s2))
    b2 = _csub(B, _cscale(B, t3, s2), _cscale(B, t4, s1))
    ib1, ib2 = _cmuli(B, b1), _cmuli(B, b2)
    return [x0, _csub(B, a1, ib1), _csub(B, a2, ib2), _cadd(B, a2, ib2), _cadd(B, a1, ib1)]


_BINS = [(k2, k1) for k2 in (1, 2, 3) for k1 in range(5)] + [(0, 1), (0, 2), (4, 1), (4, 2)]
_NCB = len(_BINS)


def _spectrum(B, x):
    z = [_rdft8(B, [x[(8 * n1 + 5 * n2) % NF] for n2 in range(8)]) for n1 in range(5)]
    for row in z:
        for c in row:
            for term in c:
                if term is not None and term[1].op != "in":
                    B.cut[term[1].idx] = term[1]
    X = [_cdft5(B, [z[n1][k2] for n1 in range(5)]) for k2 in range(5)]
    o = []
    for k2, k1 in _BINS:
        o += [X[k2][k1][0], X[k2][k1][1]]
    return o + [X[0][0][0], X[4][0][0]]


def data_program():
    B = _Prog()
    o = _spectrum(B, [B.inp(i) for i in range(NF)])
    outs = []
    for f in range(_NCB):
        outs += [B.add(o[2 * f], o[2 * f + 1]), o[2 * f], o[2 * f + 1]]
    outs += [None, o[2 * _NCB], o[2 * _NCB + 1]]
    return B, outs


def weight_program(ntaps):
    B = _Prog()
    o = _spectrum(B, [B.inp(i) if i < ntaps else None for i in range(NF)])
    outs = []
    for f in range(_NCB):
        vr, vi = o[2 * f], B.neg(o[2 * f + 1])
        outs += [vr, B.sub(vi, vr), B.add(vr, vi)]
    outs += [None, B.mul(o[2 * _NCB], 0.5), B.mul(o[2 * _NCB + 1], -0.5)]
    return B, outs


def output_program(nout):
    F = _Prog()
    o = _spectrum(F, [F.inp(i) if i < nout else None for i in range(NF)])
    B = _Prog()
    order = list(range(2 * _NCB)) + [2 * _NCB + 1, 2 * _NCB]
    adj = {}

    def push(term, val):
        if term is None or val is None:
            return
        adj.setdefault(term[1].idx, []).append(val if term[0] > 0 else B.neg(val))

    for slot, k in enumerate(order):
        push(o[k], B.inp(slot))
    res = [None] * nout
    for n in reversed(F.nodes):
        terms = adj.get(n.idx)
        if not terms:
            continue
        a = terms[0]
        for t in terms[1:]:
            a = B.add(a, t)
        if n.idx in F.cut and a[1].op != "in":
            B.cut[a[1].idx] = a[1]
        if n.op == "in":
            res[n.c] = a
        elif n.op == "add":
            push((1, n.args[0]), a); push((1, n.args[1]), a)
        elif n.op == "sub":
            push((1, n.args[0]), a); push((-1, n.args[1]), a)
        else:
            push((1, n.args[0]), B.mul(a, n.c))
    return B, res


def linearize(prog):
    B, outs = prog
    order, seen, where = [], set(), {}

    def visit(n):
        if n.idx in seen:
            return
        seen.add(n.idx)
        for a in n.args:
            visit(a)
        order.append(n)

    for k, o in enumerate(outs):
        if o is not None:
            visit(o[1])
            where.setdefault(o[1].idx, []).append((k, o[0]))
    return order, where


def staged(prog, groups):
    B, outs = prog
    need, seen = [], set()

    def visit(n):
        if n.idx in seen:
            return
        seen.add(n.idx)
        if n.idx in B.cut or n.op == "in":
            need.append(n)
            return
        for a in n.args:
            visit(a)

    for grp in groups:
        for k in grp:
            if outs[k] is not None:
                visit(outs[k][1])
    need.sort(key=lambda n: n.idx)
    slot = {n.idx: q for q, n in enumerate(need)}
    lin1 = linearize((B, [(1, n) for n in need]))
    lin2 = []
    for grp in groups:
        order, where, seen2 = [], {}, set()

        def v2(n):
            if n.idx in seen2:
                return
            seen2.add(n.idx)
            if n.idx in slot:
                order.append(("ld", n))
                return
            for a in n.args:
                v2(a)
            order.append(("op", n))

        for k in grp:
            if outs[k] is not None:
                v2(outs[k][1])
                where.setdefault(outs[k][1].idx, []).append((k, outs[k][0]))
        lin2.append((order, where))
    return slot, lin1, lin2


def _apply(n, vals):
    if n.op == "add":
        return vals[n.args[0].idx] + vals[n.args[1].idx]
    if n.op == "sub":
        return vals[n.args[0].idx] - vals[n.args[1].idx]
    return vals[n.args[0].idx] * n.c


def gen_program(lin, ld, emit):
    order, where = lin
    vals = {}
    for n in order:
        v = ld(n.c) if n.op == "in" else _apply(n, vals)
        vals[n.idx] = v
        for k, sg in where.get(n.idx, ()):
            emit(k, sg, v)
        yield 1


def gen_stage2(lin2, slot, ld, emit):
    order, where = lin2
    vals = {}
    for kind, n in order:
        v = ld(slot[n.idx]) if kind == "ld" else _apply(n, vals)
        vals[n.idx] = v
        for k, sg in where.get(n.idx, ()):
            emit(k, sg, v)
        yield 1


_S = 25
_M = 64
_NC = 5
_CR = _M * _S
_HR = _NC * _CR
_XW = 1616
_NS = 20
_NP = 3 * _NS
_SCALE = NF / 2

_DATA = data_program()
_OUT = output_program(_S)
_GRP = [[3 * f + c for f in range(5 * g, 5 * g + 5) for c in range(3)] for g in range(4)]
_DST = staged(_DATA, _GRP)
_WST = (staged(weight_program(16), _GRP), staged(weight_program(15), _GRP))
_OLIN = linearize(_OUT)
_DOPS = 2 * (len(_DST[1][0]) + sum(len(l[0]) for l in _DST[2]))
_WOPS = sum(2 * (len(w[1][0]) + sum(len(l[0]) for l in w[2])) for w in _WST)
_OOPS = len(_OLIN[0])


def _chain(gens):
    for g in gens:
        yield from g


def _kernel(x_hbm, w_hbm, g_ref, be_ref, o_hbm,
            xs, wc0, wc1, wc2, wc3, dc0, dc1, oc0, oc1, h0, h1, st, ab, tmp, xsem, wsem, osem, *, B, T, L):
    wcs = (wc0, wc1, wc2, wc3)
    dcs = (dc0, dc1); ocs = (oc0, oc1); hs = (h0, h1)
    NQ = B * _NC
    xw = xs.bitcast(jnp.uint32)
    h1u = h1.bitcast(jnp.uint32)
    ou = o_hbm.bitcast(jnp.uint32)
    wu = w_hbm.bitcast(jnp.uint32)
    zbox = [0]

    last_rows = T - (_NC - 1) * 2 * _CR
    full_rows = 2 * _XW

    def x_copy(q, par, lt, rows):
        b = q // _NC
        r0 = pl.multiple_of((q % _NC) * (2 * _CR), 16)
        return pltpu.make_async_copy(
            x_hbm.at[b, pl.ds(r0, rows), pl.ds(lt * 128, 128)],
            xs.at[par, lt, pl.ds(0, rows)], xsem.at[par])

    def x_start(q, par, last):
        for lt in range(4):
            x_copy(q, par, lt, last_rows if last else full_rows).start()
        if last:
            z = jnp.zeros((full_rows - last_rows, 128), jnp.bfloat16)
            for lt in range(4):
                xs[par, lt, pl.ds(last_rows, full_rows - last_rows), :] = z

    def x_wait(q, par, last):
        for lt in range(4):
            x_copy(q, par, lt, last_rows if last else full_rows).wait()
        if last:
            lw = last_rows // 2
            row = lax.broadcasted_iota(jnp.int32, (8, 128), 0)
            for lt in range(4):
                v = xw[par, lt, pl.ds(lw - 8, 8), :]
                xw[par, lt, pl.ds(lw - 8, 8), :] = jnp.where(row == 7, v & jnp.uint32(0xFFFF), v)

    def w_copy(lt, tap):
        return pltpu.make_async_copy(wu.at[tap, :, pl.ds(lt * 128, 128)],
                                     h1u.at[lt, pl.ds(pl.multiple_of(tap * 256, 8), 256)], wsem.at[lt])

    def o_copy(c, lt):
        n = min(_CR, L - c * _CR)
        return pltpu.make_async_copy(h1u.at[lt, pl.ds(c * _CR, n)],
                                     ou.at[pl.ds(c * _CR, n), 0, pl.ds(lt * 128, 128)], osem.at[0])

    def staged_unit(prog, ld_word, split, put):
        slot, lin1, lin2 = prog
        tm = tmp.at[zbox[0]]
        for hf in range(2):
            def emit(q, sg, v, hf=hf):
                tm[hf, q] = v
            yield from gen_program(lin1, lambda j, hf=hf: ld_word(j, hf), emit)
        for l2 in lin2:
            first = {}
            for hf in range(2):
                def emit(p, sg, v, hf=hf):
                    if hf == 0:
                        first[p] = v
                    else:
                        a, b = first[p], v
                        if split(p) * sg < 0:
                            a, b = -a, -b
                        put(p, pltpu.pack_elementwise([a, b], packed_dtype=jnp.bfloat16))
                yield from gen_stage2(l2, slot, lambda q, hf=hf: tm[hf, q], emit)

    def w_unit(lt, u):
        for ph in range(2):
            def ld(j, hf, ph=ph):
                wv = h1u[lt, pl.ds(pl.multiple_of((2 * j + ph) * 256 + u * 8, 8), 8), :]
                wv = (wv << 16) if hf == 0 else (wv & jnp.uint32(0xFFFF0000))
                return pltpu.bitcast(wv, jnp.float32)
            def put(p, v, ph=ph):
                wcs[lt][p, pl.ds(pl.multiple_of(ph * 256 + u * 8, 8), 8), :] = v
            yield from staged_unit(_WST[ph], ld, lambda p: _DATA[1][p][0], put)

    def d_unit(par, g, lt, ph):
        sub = xw.at[par, lt, pl.ds(pl.multiple_of(g * (16 * _S), 16), 416)]
        def ld(j, hf):
            w = sub[pl.ds(hf * _S + j, 8, stride=2 * _S), :]
            w = (w << 16) if ph == 0 else (w & jnp.uint32(0xFFFF0000))
            return pltpu.bitcast(w, jnp.float32)
        def put(p, v):
            dcs[par][p, ph * 4 + lt, pl.ds(pl.multiple_of(g * 8, 8), 8), :] = v
        yield from staged_unit(_DST, ld, lambda p: _DATA[1][p][0], put)

    def o_unit(par, b, c, g8, lt):
        oc = ocs[par]
        ld = lambda k: oc[k, lt, pl.ds(pl.multiple_of(g8 * 8, 8), 8), :]
        blk0 = c * _M + g8 * 8
        sub = hs[b].at[lt, pl.ds(pl.multiple_of(blk0 * _S, 8), 8 * _S)]
        blk = blk0 + lax.broadcasted_iota(jnp.int32, (8, 128), 0)
        nfull = L // _S
        jr = L - nfull * _S
        m_lo = jnp.where(blk <= nfull, 1.0, 0.0).astype(jnp.float32)
        m_hi = jnp.where(blk < nfull, 1.0, 0.0).astype(jnp.float32)
        acc = [None, None]
        def emit(j, sg, v):
            y = v if sg > 0 else -v
            sub[pl.ds(j, 8, stride=_S), :] = y
            ym = y * (m_lo if j < jr else m_hi)
            acc[0] = ym if acc[0] is None else acc[0] + ym
            acc[1] = ym * ym if acc[1] is None else acc[1] + ym * ym
        yield from gen_program(_OLIN, ld, emit)
        st[b, 0, lt] += acc[0]
        st[b, 1, lt] += acc[1]

    def stats(b, lts=range(4)):
        for lt in lts:
            s = jnp.sum(st[b, 0, lt], axis=0, keepdims=True) * (1.0 / L)
            q = jnp.sum(st[b, 1, lt], axis=0, keepdims=True) * (1.0 / L)
            var = jnp.maximum(q - s * s, 0.0) * (1.0 / (_SCALE * _SCALE))
            a = lax.rsqrt(var + 1e-5) * (1.0 / _SCALE) * g_ref[:, lt * 128:(lt + 1) * 128].astype(jnp.float32)
            bb = be_ref[:, lt * 128:(lt + 1) * 128].astype(jnp.float32) - s * a
            ab[b, 0, lt] = jnp.broadcast_to(a, (8, 128))
            ab[b, 1, lt] = jnp.broadcast_to(bb, (8, 128))

    def gelu_norm(b, lt, rows):
        z = hs[b][lt, rows, :] * ab[b, 0, lt] + ab[b, 1, lt]
        u = z * (0.7978845608028654 + 0.035677408136300125 * (z * z))
        return (0.5 * z) * (1.0 + jnp.tanh(u))

    def e_unit(c, lt):
        for r0 in range(0, _CR // 8, 5):
            rows = [pl.ds(pl.multiple_of(c * _CR + (r0 + r) * 8, 8), 8) for r in range(5)]
            vals = [gelu_norm(0, lt, rw) for rw in rows]
            for rw, v in zip(rows, vals):
                h0[lt, rw, :] = v
            yield 60

    def f_unit(lt, k):
        for r0 in range(0, _HR // 32, 5):
            rows = [pl.ds(pl.multiple_of(k * (_HR // 4) + (r0 + r) * 8, 8), 8) for r in range(5)]
            vals = [pltpu.pack_elementwise([h0[lt, rw, :], gelu_norm(1, lt, rw)],
                                           packed_dtype=jnp.bfloat16) for rw in rows]
            for rw, v in zip(rows, vals):
                h1u[lt, rw, :] = v
            yield 60

    def m_dots(par, slots, lts):
        dc = dcs[par]; oc = ocs[par]
        for f in slots:
            for lt in lts:
                k = []
                for c in range(3):
                    p = 3 * f + c
                    acc = None
                    for kt in range(8):
                        lhs = pltpu.bitcast(dc[p, kt], jnp.bfloat16)
                        rhs = pltpu.bitcast(wcs[lt][p, kt * 64:(kt + 1) * 64, :], jnp.bfloat16)
                        r = jnp.dot(lhs, rhs, preferred_element_type=jnp.float32)
                        acc = r if acc is None else acc + r
                        yield acc
                    k.append(acc)
                oc[2 * f, lt, pl.ds(0, _M), :] = k[0] - k[2]
                oc[2 * f + 1, lt, pl.ds(0, _M), :] = k[0] + k[1]

    FILL = 0.95

    def weave(mstream, nm, vec):
        done = [0] * len(vec)
        alive = [True] * len(vec)
        if mstream is not None:
            for k, acc in enumerate(mstream):
                pv = acc[0:8]
                frac = min(1.0, (k + 1) / (nm * FILL))
                for q, (g, tot, pin) in enumerate(vec):
                    if alive[q]:
                        pin(pv)
                    while alive[q] and done[q] < frac * tot:
                        try:
                            done[q] += next(g)
                        except StopIteration:
                            alive[q] = False
        for g, _, _ in vec:
            for _ in g:
                pass

    def pin_d(par, lt):
        def pin(v):
            xw[par, lt, pl.ds(pl.multiple_of(_XW + zbox[0], 8), 8), :] = pltpu.bitcast(v, jnp.uint32)
            tmp[zbox[0], 0, NF] = v
        return pin

    def pin_w(lt):
        def pin(v):
            h1[lt, pl.ds(pl.multiple_of(_HR + zbox[0], 8), 8), :] = v
            tmp[zbox[0], 0, NF] = v
        return pin

    def pin_o(par, lt):
        def pin(v):
            ocs[par][0, lt, pl.ds(pl.multiple_of(_M + zbox[0], 8), 8), :] = v
        return pin

    def pin_e(lt):
        def pin(v):
            h0[lt, pl.ds(pl.multiple_of(_HR + zbox[0], 8), 8), :] = v
        return pin

    def d_lt(par, lt):
        return (_chain(d_unit(par, k // 2, lt, k % 2) for k in range(8)), 8 * _DOPS, pin_d(par, lt))

    def o_lt(par, b, c, lt):
        return (_chain(o_unit(par, b, c, g8, lt) for g8 in range(8)), 8 * _OOPS, pin_o(par, lt))

    def e_lt(c, lt):
        return (e_unit(c, lt), 12 * (_CR // 8), pin_e(lt))

    def w_part(lt, u0, n):
        return (_chain(w_unit(lt, u0 + k) for k in range(n)), n * _WOPS, pin_w(lt))

    def step(t, par, D, Mm, O, E, ob):
        def body(i, carry):
            zbox[0] = i // 64
            vec = []
            if D:
                vec.append(d_lt(par, i))
            if O:
                vec.append(o_lt(par, ob, t - 2 - ob * _NC, i))
            if E:
                vec.append(e_lt(t - (_NC + 2), i))
            ms = m_dots(1 - par, [5 * i + k for k in range(5)], range(4)) if Mm else None
            weave(ms, 480, vec)
            return carry
        lax.fori_loop(0, 4, body, 0)

    for tap in range(31):
        w_copy(0, tap).start()
    x_start(0, 0, False)
    x_start(1, 1, False)
    st[...] = jnp.zeros(st.shape, jnp.float32)
    zc = jnp.zeros((512, 128), jnp.uint32)
    for lt in range(4):
        wcs[lt][_NP - 3] = zc
    zd = jnp.zeros((_M // 2, 128), jnp.uint32)
    for dc in dcs:
        for kt in range(8):
            dc[_NP - 3, kt] = zd

    def w_wait(lt):
        for tap in range(31):
            w_copy(lt, tap).wait()

    w_wait(0)
    def w0_body(u, c):
        zbox[0] = u // 64
        for lt in range(1, 4):
            w_copy(lt, 2 * u).start()
            @pl.when(u < 15)
            def _():
                w_copy(lt, 2 * u + 1).start()
        weave(None, 0, [w_part(0, 2 * u, 2)])
        return c
    lax.fori_loop(0, 16, w0_body, 0)
    for par in range(2):
        x_wait(par, par, False)
        def d0_body(i, c, par=par):
            zbox[0] = i // 64
            weave(None, 0, [d_lt(par, i)])
            return c
        lax.fori_loop(0, 4, d0_body, 0)

    for lt in range(3):
        w_wait(lt + 1)
        for par in range(2):
            def inner(k, c2, par=par, lt=lt):
                zbox[0] = k // 64
                weave(m_dots(par, [5 * k + j for j in range(5)], [lt]), 120,
                      [w_part(lt + 1, 16 * par + 4 * k, 4)])
                return c2
            lax.fori_loop(0, 4, inner, 0)

    x_start(2, 0, False)
    def last0(k, c):
        zbox[0] = k // 64
        weave(m_dots(0, [5 * k + j for j in range(5)], [3]), 120, [])
        return c
    lax.fori_loop(0, 4, last0, 0)
    x_wait(2, 0, False)
    x_start(3, 1, False)
    def last1(k, c):
        zbox[0] = k // 64
        weave(m_dots(1, [5 * k + j for j in range(5)], [3]), 120, [d_lt(0, k), o_lt(0, 0, 0, k)])
        return c
    lax.fori_loop(0, 4, last1, 0)

    def advance(t, par, last_now, last_next):
        x_wait(t, par, last_now)
        if last_next is not None:
            x_start(t + 1, 1 - par, last_next)

    def pair(k, c):
        t = 3 + 2 * k
        advance(t, 1, False, None)
        @pl.when(k == 0)
        def _():
            x_start(t + 1, 0, True)
        @pl.when(k != 0)
        def _():
            x_start(t + 1, 0, False)
        step(t, 1, True, True, True, False, 0)
        @pl.when(k == 0)
        def _():
            x_wait(t + 1, 0, True)
        @pl.when(k != 0)
        def _():
            x_wait(t + 1, 0, False)
        x_start(t + 2, 1, False)
        step(t + 1, 0, True, True, True, False, 0)
        return c
    lax.fori_loop(0, 2, pair, 0)
    stats(0)
    advance(7, 1, False, False)
    step(7, 1, True, True, True, True, 1)
    advance(8, 0, False, True)
    step(8, 0, True, True, True, True, 1)
    x_wait(9, 1, True)

    def block(par, lt, make_vec):
        def body(k, c):
            zbox[0] = k // 64
            weave(m_dots(par, [5 * k + j for j in range(5)], [lt]), 120, make_vec(k))
            return c
        lax.fori_loop(0, 4, body, 0)

    def o_pair(lt, k):
        return [(_chain([o_unit(par, 1, 3 + par, 2 * k + j, lt) for j in range(2)]), 2 * _OOPS, pin_o(par, lt))
                for par in range(2)]

    def f_vec(lt, k):
        return [(f_unit(lt, k), 12 * (_HR // 32), pin_f(lt))]

    def pin_f(lt):
        def pin(v):
            h0[lt, pl.ds(pl.multiple_of(_HR + zbox[0], 8), 8), :] = v
            h1[lt, pl.ds(pl.multiple_of(_HR + zbox[0], 8), 8), :] = v
        return pin

    def out_start(lt):
        for cch in range(_NC):
            o_copy(cch, lt).start()

    block(0, 0, lambda k: [d_lt(1, k), o_lt(1, 1, 2, k)])
    block(1, 0, lambda k: [e_lt(2, k), e_lt(3, k), e_lt(4, k)])
    for lt in range(1, 4):
        block(0, lt, lambda k, lt=lt: o_pair(lt - 1, k))
        stats(1, [lt - 1])
        block(1, lt, lambda k, lt=lt: f_vec(lt - 1, k))
        out_start(lt - 1)

    def tail(make_vec):
        def body(k, c):
            zbox[0] = k // 64
            weave(None, 0, make_vec(k))
            return c
        lax.fori_loop(0, 4, body, 0)

    tail(lambda k: o_pair(3, k))
    stats(1, [3])
    tail(lambda k: f_vec(3, k))
    out_start(3)
    for lt in range(4):
        for cch in range(_NC):
            o_copy(cch, lt).wait()


@jax.jit
def pallas_standalone__self_sup_conv_stem_wavlm__speech_kernel(x, w, gn_gamma, gn_beta):
    B, T, D = x.shape
    K = w.shape[0]
    L = (T - K) // 2 + 1
    assert (B, T, D, K) == (2, 16000, 512, 31)
    out = pl.pallas_call(
        functools.partial(_kernel, B=B, T=T, L=L),
        grid=(1,),
        in_specs=[
            pl.BlockSpec(memory_space=pl.ANY),
            pl.BlockSpec(memory_space=pl.ANY),
            pl.BlockSpec((1, D), lambda t: (0, 0)),
            pl.BlockSpec((1, D), lambda t: (0, 0)),
        ],
        out_specs=pl.BlockSpec(memory_space=pl.ANY),
        out_shape=jax.ShapeDtypeStruct((L, B, D), jnp.bfloat16),
        scratch_shapes=[
            pltpu.VMEM((2, 4, 2 * _XW + 16, 128), jnp.bfloat16),
            *[pltpu.VMEM((_NP, D, 128), jnp.uint32) for _ in range(4)],
            pltpu.VMEM((_NP, 8, _M // 2, 128), jnp.uint32),
            pltpu.VMEM((_NP, 8, _M // 2, 128), jnp.uint32),
            pltpu.VMEM((NF, 4, _M + 8, 128), jnp.float32),
            pltpu.VMEM((NF, 4, _M + 8, 128), jnp.float32),
            pltpu.VMEM((4, _HR + 8, 128), jnp.float32),
            pltpu.VMEM((4, _HR + 8, 128), jnp.float32),
            pltpu.VMEM((B, 2, 4, 8, 128), jnp.float32),
            pltpu.VMEM((B, 2, 4, 8, 128), jnp.float32),
            pltpu.VMEM((1, 2, NF + 1, 8, 128), jnp.float32),
            pltpu.SemaphoreType.DMA((2,)),
            pltpu.SemaphoreType.DMA((4,)),
            pltpu.SemaphoreType.DMA((1,)),
        ],
        compiler_params=pltpu.CompilerParams(
            dimension_semantics=("arbitrary",),
            vmem_limit_bytes=127 * 1024 * 1024,
        ),
    )(x, w, gn_gamma.reshape(1, D), gn_beta.reshape(1, D))
    return jnp.transpose(out, (1, 0, 2))
```

```python
import math
import functools
import jax
import jax.numpy as jnp
from jax import lax
from jax.experimental import pallas as pl
from jax.experimental.pallas import tpu as pltpu

NF = 40


class _Node:
    __slots__ = ("op", "args", "c", "idx")


class _Prog:
    def __init__(self):
        self.nodes = []
        self.cse = {}
        self.cut = {}

    def _mk(self, op, args=(), c=None):
        key = (op, tuple(a.idx for a in args), c)
        n = self.cse.get(key)
        if n is None:
            n = _Node()
            n.op, n.args, n.c, n.idx = op, args, c, len(self.nodes)
            self.nodes.append(n)
            self.cse[key] = n
        return n

    def inp(self, i):
        return (1, self._mk("in", (), i))

    def neg(self, a):
        return None if a is None else (-a[0], a[1])

    def add(self, a, b):
        if a is None:
            return b
        if b is None:
            return a
        (sa, na), (sb, nb) = a, b
        if sa == sb:
            if na is nb:
                return (sa, self._mk("mul", (na,), 2.0))
            x, y = sorted((na, nb), key=lambda n: n.idx)
            return (sa, self._mk("add", (x, y)))
        if na is nb:
            return None
        if sa > 0:
            return (1, self._mk("sub", (na, nb)))
        return (1, self._mk("sub", (nb, na)))

    def sub(self, a, b):
        return self.add(a, self.neg(b))

    def mul(self, a, c):
        if a is None or abs(c) < 1e-12:
            return None
        if abs(c - 1) < 1e-12:
            return a
        if abs(c + 1) < 1e-12:
            return self.neg(a)
        return (a[0] * (1 if c > 0 else -1), self._mk("mul", (a[1],), abs(float(c))))


def _cadd(B, a, b): return (B.add(a[0], b[0]), B.add(a[1], b[1]))
def _csub(B, a, b): return (B.sub(a[0], b[0]), B.sub(a[1], b[1]))
def _cscale(B, a, c): return (B.mul(a[0], c), B.mul(a[1], c))
def _cconj(B, a): return (a[0], B.neg(a[1]))
def _cmuli(B, a): return (B.neg(a[1]), a[0])


def _rdft8(B, x):
    a0, a1 = B.add(x[0], x[4]), B.sub(x[0], x[4])
    b0, b1 = B.add(x[2], x[6]), B.sub(x[2], x[6])
    c0, c1 = B.add(x[1], x[5]), B.sub(x[1], x[5])
    d0, d1 = B.add(x[3], x[7]), B.sub(x[3], x[7])
    e0, e2 = B.add(a0, b0), B.sub(a0, b0)
    o0, o2 = B.add(c0, d0), B.sub(c0, d0)
    r = math.sqrt(0.5)
    p = B.mul(B.sub(c1, d1), r)
    q = B.mul(B.add(c1, d1), r)
    return [
        (B.add(e0, o0), None),
        (B.add(a1, p), B.neg(B.add(b1, q))),
        (e2, B.neg(o2)),
        (B.sub(a1, p), B.sub(b1, q)),
        (B.sub(e0, o0), None),
    ]


def _cdft5(B, z):
    t1, t2 = _cadd(B, z[1], z[4]), _cadd(B, z[2], z[3])
    t3, t4 = _csub(B, z[1], z[4]), _csub(B, z[2], z[3])
    m = _cadd(B, t1, t2)
    x0 = _cadd(B, z[0], m)
    u = _csub(B, z[0], _cscale(B, m, 0.25))
    v = _cscale(B, _csub(B, t1, t2), math.sqrt(5.0) / 4.0)
    a1, a2 = _cadd(B, u, v), _csub(B, u, v)
    s1, s2 = math.sin(2 * math.pi / 5), math.sin(4 * math.pi / 5)
    b1 = _cadd(B, _cscale(B, t3, s1), _cscale(B, t4, s2))
    b2 = _csub(B, _cscale(B, t3, s2), _cscale(B, t4, s1))
    ib1, ib2 = _cmuli(B, b1), _cmuli(B, b2)
    return [x0, _csub(B, a1, ib1), _csub(B, a2, ib2), _cadd(B, a2, ib2), _cadd(B, a1, ib1)]


_BINS = [(k2, k1) for k2 in (1, 2, 3) for k1 in range(5)] + [(0, 1), (0, 2), (4, 1), (4, 2)]
_NCB = len(_BINS)


def _spectrum(B, x):
    z = [_rdft8(B, [x[(8 * n1 + 5 * n2) % NF] for n2 in range(8)]) for n1 in range(5)]
    for row in z:
        for c in row:
            for term in c:
                if term is not None and term[1].op != "in":
                    B.cut[term[1].idx] = term[1]
    X = [_cdft5(B, [z[n1][k2] for n1 in range(5)]) for k2 in range(5)]
    o = []
    for k2, k1 in _BINS:
        o += [X[k2][k1][0], X[k2][k1][1]]
    return o + [X[0][0][0], X[4][0][0]]


def data_program():
    B = _Prog()
    o = _spectrum(B, [B.inp(i) for i in range(NF)])
    outs = []
    for f in range(_NCB):
        outs += [B.add(o[2 * f], o[2 * f + 1]), o[2 * f], o[2 * f + 1]]
    outs += [None, o[2 * _NCB], o[2 * _NCB + 1]]
    return B, outs


def weight_program(ntaps):
    B = _Prog()
    o = _spectrum(B, [B.inp(i) if i < ntaps else None for i in range(NF)])
    outs = []
    for f in range(_NCB):
        vr, vi = o[2 * f], B.neg(o[2 * f + 1])
        outs += [vr, B.sub(vi, vr), B.add(vr, vi)]
    outs += [None, B.mul(o[2 * _NCB], 0.5), B.mul(o[2 * _NCB + 1], -0.5)]
    return B, outs


def output_program(nout):
    F = _Prog()
    o = _spectrum(F, [F.inp(i) if i < nout else None for i in range(NF)])
    B = _Prog()
    order = list(range(2 * _NCB)) + [2 * _NCB + 1, 2 * _NCB]
    adj = {}

    def push(term, val):
        if term is None or val is None:
            return
        adj.setdefault(term[1].idx, []).append(val if term[0] > 0 else B.neg(val))

    for slot, k in enumerate(order):
        push(o[k], B.inp(slot))
    res = [None] * nout
    for n in reversed(F.nodes):
        terms = adj.get(n.idx)
        if not terms:
            continue
        a = terms[0]
        for t in terms[1:]:
            a = B.add(a, t)
        if n.idx in F.cut and a[1].op != "in":
            B.cut[a[1].idx] = a[1]
        if n.op == "in":
            res[n.c] = a
        elif n.op == "add":
            push((1, n.args[0]), a); push((1, n.args[1]), a)
        elif n.op == "sub":
            push((1, n.args[0]), a); push((-1, n.args[1]), a)
        else:
            push((1, n.args[0]), B.mul(a, n.c))
    return B, res


def linearize(prog):
    B, outs = prog
    order, seen, where = [], set(), {}

    def visit(n):
        if n.idx in seen:
            return
        seen.add(n.idx)
        for a in n.args:
            visit(a)
        order.append(n)

    for k, o in enumerate(outs):
        if o is not None:
            visit(o[1])
            where.setdefault(o[1].idx, []).append((k, o[0]))
    return order, where


def staged(prog, groups):
    B, outs = prog
    need, seen = [], set()

    def visit(n):
        if n.idx in seen:
            return
        seen.add(n.idx)
        if n.idx in B.cut or n.op == "in":
            need.append(n)
            return
        for a in n.args:
            visit(a)

    for grp in groups:
        for k in grp:
            if outs[k] is not None:
                visit(outs[k][1])
    need.sort(key=lambda n: n.idx)
    slot = {n.idx: q for q, n in enumerate(need)}
    lin1 = linearize((B, [(1, n) for n in need]))
    lin2 = []
    for grp in groups:
        order, where, seen2 = [], {}, set()

        def v2(n):
            if n.idx in seen2:
                return
            seen2.add(n.idx)
            if n.idx in slot:
                order.append(("ld", n))
                return
            for a in n.args:
                v2(a)
            order.append(("op", n))

        for k in grp:
            if outs[k] is not None:
                v2(outs[k][1])
                where.setdefault(outs[k][1].idx, []).append((k, outs[k][0]))
        lin2.append((order, where))
    return slot, lin1, lin2


def _apply(n, vals):
    if n.op == "add":
        return vals[n.args[0].idx] + vals[n.args[1].idx]
    if n.op == "sub":
        return vals[n.args[0].idx] - vals[n.args[1].idx]
    return vals[n.args[0].idx] * n.c


def gen_program(lin, ld, emit):
    order, where = lin
    vals = {}
    for n in order:
        v = ld(n.c) if n.op == "in" else _apply(n, vals)
        vals[n.idx] = v
        for k, sg in where.get(n.idx, ()):
            emit(k, sg, v)
        yield 1


def gen_stage2(lin2, slot, ld, emit):
    order, where = lin2
    vals = {}
    for kind, n in order:
        v = ld(slot[n.idx]) if kind == "ld" else _apply(n, vals)
        vals[n.idx] = v
        for k, sg in where.get(n.idx, ()):
            emit(k, sg, v)
        yield 1


_S = 25
_M = 64
_NC = 5
_CR = _M * _S
_HR = _NC * _CR
_XW = 1616
_NS = 20
_NP = 3 * _NS
_SCALE = NF / 2

_DATA = data_program()
_OUT = output_program(_S)
_GRP = [[3 * f + c for f in range(5 * g, 5 * g + 5) for c in range(3)] for g in range(4)]
_DST = staged(_DATA, _GRP)
_WST = (staged(weight_program(16), _GRP), staged(weight_program(15), _GRP))
_OLIN = linearize(_OUT)
_DOPS = 2 * (len(_DST[1][0]) + sum(len(l[0]) for l in _DST[2]))
_WOPS = sum(2 * (len(w[1][0]) + sum(len(l[0]) for l in w[2])) for w in _WST)
_OOPS = len(_OLIN[0])


def _chain(gens):
    for g in gens:
        yield from g


def _kernel(x_hbm, w_hbm, g_ref, be_ref, o_hbm,
            xs, wc0, wc1, wc2, wc3, dc0, dc1, oc0, oc1, h0, h1, st, ab, tmp, xsem, wsem, osem, *, B, T, L):
    wcs = (wc0, wc1, wc2, wc3)
    dcs = (dc0, dc1); ocs = (oc0, oc1); hs = (h0, h1)
    NQ = B * _NC
    xw = xs.bitcast(jnp.uint32)
    h1u = h1.bitcast(jnp.uint32)
    ou = o_hbm.bitcast(jnp.uint32)
    wu = w_hbm.bitcast(jnp.uint32)
    zbox = [0]

    last_rows = T - (_NC - 1) * 2 * _CR
    full_rows = 2 * _XW

    def x_copy(q, par, lt, rows):
        b = q // _NC
        r0 = pl.multiple_of((q % _NC) * (2 * _CR), 16)
        return pltpu.make_async_copy(
            x_hbm.at[b, pl.ds(r0, rows), pl.ds(lt * 128, 128)],
            xs.at[par, lt, pl.ds(0, rows)], xsem.at[par])

    def x_start(q, par, last):
        for lt in range(4):
            x_copy(q, par, lt, last_rows if last else full_rows).start()
        if last:
            z = jnp.zeros((full_rows - last_rows, 128), jnp.bfloat16)
            for lt in range(4):
                xs[par, lt, pl.ds(last_rows, full_rows - last_rows), :] = z

    def x_wait(q, par, last):
        for lt in range(4):
            x_copy(q, par, lt, last_rows if last else full_rows).wait()
        if last:
            lw = last_rows // 2
            row = lax.broadcasted_iota(jnp.int32, (8, 128), 0)
            for lt in range(4):
                v = xw[par, lt, pl.ds(lw - 8, 8), :]
                xw[par, lt, pl.ds(lw - 8, 8), :] = jnp.where(row == 7, v & jnp.uint32(0xFFFF), v)

    def w_copy(lt, tap):
        return pltpu.make_async_copy(wu.at[tap, :, pl.ds(lt * 128, 128)],
                                     h1u.at[lt, pl.ds(pl.multiple_of(tap * 256, 8), 256)], wsem.at[lt])

    def o_copy(c, lt):
        n = min(_CR, L - c * _CR)
        return pltpu.make_async_copy(h1u.at[lt, pl.ds(c * _CR, n)],
                                     ou.at[pl.ds(c * _CR, n), 0, pl.ds(lt * 128, 128)], osem.at[0])

    def staged_unit(prog, ld_word, split, put):
        slot, lin1, lin2 = prog
        tm = tmp.at[zbox[0]]
        for hf in range(2):
            def emit(q, sg, v, hf=hf):
                tm[hf, q] = v
            yield from gen_program(lin1, lambda j, hf=hf: ld_word(j, hf), emit)
        for l2 in lin2:
            first = {}
            for hf in range(2):
                def emit(p, sg, v, hf=hf):
                    if hf == 0:
                        first[p] = v
                    else:
                        a, b = first[p], v
                        if split(p) * sg < 0:
                            a, b = -a, -b
                        put(p, pltpu.pack_elementwise([a, b], packed_dtype=jnp.bfloat16))
                yield from gen_stage2(l2, slot, lambda q, hf=hf: tm[hf, q], emit)

    def w_unit(lt, u):
        for ph in range(2):
            def ld(j, hf, ph=ph):
                wv = h1u[lt, pl.ds(pl.multiple_of((2 * j + ph) * 256 + u * 8, 8), 8), :]
                wv = (wv << 16) if hf == 0 else (wv & jnp.uint32(0xFFFF0000))
                return pltpu.bitcast(wv, jnp.float32)
            def put(p, v, ph=ph):
                wcs[lt][p, pl.ds(pl.multiple_of(ph * 256 + u * 8, 8), 8), :] = v
            yield from staged_unit(_WST[ph], ld, lambda p: _DATA[1][p][0], put)

    def d_unit(par, g, lt, ph):
        sub = xw.at[par, lt, pl.ds(pl.multiple_of(g * (16 * _S), 16), 416)]
        def ld(j, hf):
            w = sub[pl.ds(hf * _S + j, 8, stride=2 * _S), :]
            w = (w << 16) if ph == 0 else (w & jnp.uint32(0xFFFF0000))
            return pltpu.bitcast(w, jnp.float32)
        def put(p, v):
            dcs[par][p, ph * 4 + lt, pl.ds(pl.multiple_of(g * 8, 8), 8), :] = v
        yield from staged_unit(_DST, ld, lambda p: _DATA[1][p][0], put)

    def o_unit(par, b, c, g8, lt):
        oc = ocs[par]
        ld = lambda k: oc[k, lt, pl.ds(pl.multiple_of(g8 * 8, 8), 8), :]
        blk0 = c * _M + g8 * 8
        sub = hs[b].at[lt, pl.ds(pl.multiple_of(blk0 * _S, 8), 8 * _S)]
        blk = blk0 + lax.broadcasted_iota(jnp.int32, (8, 128), 0)
        nfull = L // _S
        jr = L - nfull * _S
        m_lo = jnp.where(blk <= nfull, 1.0, 0.0).astype(jnp.float32)
        m_hi = jnp.where(blk < nfull, 1.0, 0.0).astype(jnp.float32)
        acc = [None, None]
        def emit(j, sg, v):
            y = v if sg > 0 else -v
            sub[pl.ds(j, 8, stride=_S), :] = y
            ym = y * (m_lo if j < jr else m_hi)
            acc[0] = ym if acc[0] is None else acc[0] + ym
            acc[1] = ym * ym if acc[1] is None else acc[1] + ym * ym
        yield from gen_program(_OLIN, ld, emit)
        st[b, 0, lt] += acc[0]
        st[b, 1, lt] += acc[1]

    def stats(b, lts=range(4)):
        for lt in lts:
            s = jnp.sum(st[b, 0, lt], axis=0, keepdims=True) * (1.0 / L)
            q = jnp.sum(st[b, 1, lt], axis=0, keepdims=True) * (1.0 / L)
            var = jnp.maximum(q - s * s, 0.0) * (1.0 / (_SCALE * _SCALE))
            a = lax.rsqrt(var + 1e-5) * (1.0 / _SCALE) * g_ref[:, lt * 128:(lt + 1) * 128].astype(jnp.float32)
            bb = be_ref[:, lt * 128:(lt + 1) * 128].astype(jnp.float32) - s * a
            ab[b, 0, lt] = jnp.broadcast_to(a, (8, 128))
            ab[b, 1, lt] = jnp.broadcast_to(bb, (8, 128))

    def gelu_norm(b, lt, rows):
        z = hs[b][lt, rows, :] * ab[b, 0, lt] + ab[b, 1, lt]
        u = z * (0.7978845608028654 + 0.035677408136300125 * (z * z))
        return (0.5 * z) * (1.0 + jnp.tanh(u))

    def e_unit(c, lt):
        for r0 in range(0, _CR // 8, 5):
            rows = [pl.ds(pl.multiple_of(c * _CR + (r0 + r) * 8, 8), 8) for r in range(5)]
            vals = [gelu_norm(0, lt, rw) for rw in rows]
            for rw, v in zip(rows, vals):
                h0[lt, rw, :] = v
            yield 60

    def f_unit(lt, k):
        for r0 in range(0, _HR // 32, 5):
            rows = [pl.ds(pl.multiple_of(k * (_HR // 4) + (r0 + r) * 8, 8), 8) for r in range(5)]
            vals = [pltpu.pack_elementwise([h0[lt, rw, :], gelu_norm(1, lt, rw)],
                                           packed_dtype=jnp.bfloat16) for rw in rows]
            for rw, v in zip(rows, vals):
                h1u[lt, rw, :] = v
            yield 60

    def m_dots(par, slots, lts):
        dc = dcs[par]; oc = ocs[par]
        for f in slots:
            for lt in lts:
                k = []
                for c in range(3):
                    p = 3 * f + c
                    acc = None
                    for kt in range(8):
                        lhs = pltpu.bitcast(dc[p, kt], jnp.bfloat16)
                        rhs = pltpu.bitcast(wcs[lt][p, kt * 64:(kt + 1) * 64, :], jnp.bfloat16)
                        r = jnp.dot(lhs, rhs, preferred_element_type=jnp.float32)
                        acc = r if acc is None else acc + r
                        yield acc
                    k.append(acc)
                oc[2 * f, lt, pl.ds(0, _M), :] = k[0] - k[2]
                oc[2 * f + 1, lt, pl.ds(0, _M), :] = k[0] + k[1]

    FILL = 0.95
    F1 = 1.0
    F2 = 0.85
    PR = 0
    PE = 1

    def weave(mstream, nm, vec, fill=FILL):
        done = [0] * len(vec)
        alive = [True] * len(vec)
        if mstream is not None:
            for k, acc in enumerate(mstream):
                pv = acc[PR:PR + 8]
                frac = min(1.0, (k + 1) / (nm * fill))
                for q, (g, tot, pin) in enumerate(vec):
                    if alive[q] and k % PE == PE - 1:
                        pin(pv)
                    while alive[q] and done[q] < frac * tot:
                        try:
                            done[q] += next(g)
                        except StopIteration:
                            alive[q] = False
        for g, _, _ in vec:
            for _ in g:
                pass

    def pin_d(par, lt):
        def pin(v):
            xw[par, lt, pl.ds(pl.multiple_of(_XW + zbox[0], 8), 8), :] = pltpu.bitcast(v, jnp.uint32)
            tmp[zbox[0], 0, NF] = v
        return pin

    def pin_w(lt):
        def pin(v):
            h1[lt, pl.ds(pl.multiple_of(_HR + zbox[0], 8), 8), :] = v
            tmp[zbox[0], 0, NF] = v
        return pin

    def pin_o(par, lt):
        def pin(v):
            ocs[par][0, lt, pl.ds(pl.multiple_of(_M + zbox[0], 8), 8), :] = v
        return pin

    def pin_e(lt):
        def pin(v):
            h0[lt, pl.ds(pl.multiple_of(_HR + zbox[0], 8), 8), :] = v
        return pin

    def d_lt(par, lt):
        return (_chain(d_unit(par, k // 2, lt, k % 2) for k in range(8)), 8 * _DOPS, pin_d(par, lt))

    def o_lt(par, b, c, lt):
        return (_chain(o_unit(par, b, c, g8, lt) for g8 in range(8)), 8 * _OOPS, pin_o(par, lt))

    def e_lt(c, lt):
        return (e_unit(c, lt), 12 * (_CR // 8), pin_e(lt))

    def w_part(lt, u0, n):
        return (_chain(w_unit(lt, u0 + k) for k in range(n)), n * _WOPS, pin_w(lt))

    def step(t, par, D, Mm, O, E, ob):
        def body(i, carry):
            zbox[0] = i // 64
            vec = []
            if D:
                vec.append(d_lt(par, i))
            if O:
                vec.append(o_lt(par, ob, t - 2 - ob * _NC, i))
            if E:
                vec.append(e_lt(2 * (t - (_NC + 2)), i))
                vec.append(e_lt(2 * (t - (_NC + 2)) + 1, i))
            ms = m_dots(1 - par, [5 * i + k for k in range(5)], range(4)) if Mm else None
            weave(ms, 480, vec, F2 if E else F1)
            return carry
        lax.fori_loop(0, 4, body, 0)

    for tap in range(31):
        w_copy(0, tap).start()
    x_start(0, 0, False)
    x_start(1, 1, False)
    st[...] = jnp.zeros(st.shape, jnp.float32)
    zc = jnp.zeros((512, 128), jnp.uint32)
    for lt in range(4):
        wcs[lt][_NP - 3] = zc
    zd = jnp.zeros((_M // 2, 128), jnp.uint32)
    for dc in dcs:
        for kt in range(8):
            dc[_NP - 3, kt] = zd

    def w_wait(lt):
        for tap in range(31):
            w_copy(lt, tap).wait()

    w_wait(0)
    def w0_body(u, c):
        zbox[0] = u // 64
        for lt in range(1, 4):
            w_copy(lt, 2 * u).start()
            @pl.when(u < 15)
            def _():
                w_copy(lt, 2 * u + 1).start()
        weave(None, 0, [w_part(0, 2 * u, 2)])
        return c
    lax.fori_loop(0, 16, w0_body, 0)
    for par in range(2):
        x_wait(par, par, False)
        def d0_body(i, c, par=par):
            zbox[0] = i // 64
            weave(None, 0, [d_lt(par, i)])
            return c
        lax.fori_loop(0, 4, d0_body, 0)

    for lt in range(3):
        w_wait(lt + 1)
        for par in range(2):
            def inner(k, c2, par=par, lt=lt):
                zbox[0] = k // 64
                weave(m_dots(par, [5 * k + j for j in range(5)], [lt]), 120,
                      [w_part(lt + 1, 16 * par + 4 * k, 4)])
                return c2
            lax.fori_loop(0, 4, inner, 0)

    x_start(2, 0, False)
    def last0(k, c):
        zbox[0] = k // 64
        weave(m_dots(0, [5 * k + j for j in range(5)], [3]), 120, [])
        return c
    lax.fori_loop(0, 4, last0, 0)
    x_wait(2, 0, False)
    x_start(3, 1, False)
    def last1(k, c):
        zbox[0] = k // 64
        weave(m_dots(1, [5 * k + j for j in range(5)], [3]), 120, [d_lt(0, k), o_lt(0, 0, 0, k)])
        return c
    lax.fori_loop(0, 4, last1, 0)

    def advance(t, par, last_now, last_next):
        x_wait(t, par, last_now)
        if last_next is not None:
            x_start(t + 1, 1 - par, last_next)

    def pair(k, c):
        t = 3 + 2 * k
        advance(t, 1, False, None)
        @pl.when(k == 0)
        def _():
            x_start(t + 1, 0, True)
        @pl.when(k != 0)
        def _():
            x_start(t + 1, 0, False)
        step(t, 1, True, True, True, False, 0)
        @pl.when(k == 0)
        def _():
            x_wait(t + 1, 0, True)
        @pl.when(k != 0)
        def _():
            x_wait(t + 1, 0, False)
        x_start(t + 2, 1, False)
        step(t + 1, 0, True, True, True, False, 0)
        return c
    lax.fori_loop(0, 2, pair, 0)
    stats(0)
    advance(7, 1, False, False)
    step(7, 1, True, True, True, True, 1)
    advance(8, 0, False, True)
    step(8, 0, True, True, True, True, 1)
    x_wait(9, 1, True)

    def block(par, lt, make_vec):
        def body(k, c):
            zbox[0] = k // 64
            weave(m_dots(par, [5 * k + j for j in range(5)], [lt]), 120, make_vec(k))
            return c
        lax.fori_loop(0, 4, body, 0)

    def o_pair(lt, k):
        return [(_chain([o_unit(par, 1, 3 + par, 2 * k + j, lt) for j in range(2)]), 2 * _OOPS, pin_o(par, lt))
                for par in range(2)]

    def f_vec(lt, k):
        return [(f_unit(lt, k), 12 * (_HR // 32), pin_f(lt))]

    def pin_f(lt):
        def pin(v):
            h0[lt, pl.ds(pl.multiple_of(_HR + zbox[0], 8), 8), :] = v
            h1[lt, pl.ds(pl.multiple_of(_HR + zbox[0], 8), 8), :] = v
        return pin

    def out_start(lt):
        for cch in range(_NC):
            o_copy(cch, lt).start()

    block(0, 0, lambda k: [d_lt(1, k), o_lt(1, 1, 2, k)])
    block(1, 0, lambda k: [e_lt(4, k)])
    for lt in range(1, 4):
        block(0, lt, lambda k, lt=lt: o_pair(lt - 1, k))
        stats(1, [lt - 1])
        block(1, lt, lambda k, lt=lt: f_vec(lt - 1, k))
        out_start(lt - 1)

    def tail(make_vec):
        def body(k, c):
            zbox[0] = k // 64
            weave(None, 0, make_vec(k))
            return c
        lax.fori_loop(0, 4, body, 0)

    tail(lambda k: o_pair(3, k))
    stats(1, [3])
    tail(lambda k: f_vec(3, k))
    out_start(3)
    for lt in range(4):
        for cch in range(_NC):
            o_copy(cch, lt).wait()


@jax.jit
def pallas_standalone__self_sup_conv_stem_wavlm__speech_kernel(x, w, gn_gamma, gn_beta):
    B, T, D = x.shape
    K = w.shape[0]
    L = (T - K) // 2 + 1
    assert (B, T, D, K) == (2, 16000, 512, 31)
    out = pl.pallas_call(
        functools.partial(_kernel, B=B, T=T, L=L),
        grid=(1,),
        in_specs=[
            pl.BlockSpec(memory_space=pl.ANY),
            pl.BlockSpec(memory_space=pl.ANY),
            pl.BlockSpec((1, D), lambda t: (0, 0)),
            pl.BlockSpec((1, D), lambda t: (0, 0)),
        ],
        out_specs=pl.BlockSpec(memory_space=pl.ANY),
        out_shape=jax.ShapeDtypeStruct((L, B, D), jnp.bfloat16),
        scratch_shapes=[
            pltpu.VMEM((2, 4, 2 * _XW + 16, 128), jnp.bfloat16),
            *[pltpu.VMEM((_NP, D, 128), jnp.uint32) for _ in range(4)],
            pltpu.VMEM((_NP, 8, _M // 2, 128), jnp.uint32),
            pltpu.VMEM((_NP, 8, _M // 2, 128), jnp.uint32),
            pltpu.VMEM((NF, 4, _M + 8, 128), jnp.float32),
            pltpu.VMEM((NF, 4, _M + 8, 128), jnp.float32),
            pltpu.VMEM((4, _HR + 8, 128), jnp.float32),
            pltpu.VMEM((4, _HR + 8, 128), jnp.float32),
            pltpu.VMEM((B, 2, 4, 8, 128), jnp.float32),
            pltpu.VMEM((B, 2, 4, 8, 128), jnp.float32),
            pltpu.VMEM((1, 2, NF + 1, 8, 128), jnp.float32),
            pltpu.SemaphoreType.DMA((2,)),
            pltpu.SemaphoreType.DMA((4,)),
            pltpu.SemaphoreType.DMA((1,)),
        ],
        compiler_params=pltpu.CompilerParams(
            dimension_semantics=("arbitrary",),
            vmem_limit_bytes=127 * 1024 * 1024,
        ),
    )(x, w, gn_gamma.reshape(1, D), gn_beta.reshape(1, D))
    return jnp.transpose(out, (1, 0, 2))
```
